```python
import jax
import jax.numpy as jnp

def _softmax(x, axis=-1):
    return jax.nn.softmax(x, axis=axis)
def _gelu(x):
    return jax.nn.gelu(x, approximate=True)
def _silu(x):
    return jax.nn.silu(x)
def _sigmoid(x):
    return jax.nn.sigmoid(x)
def _layernorm(x, axis=-1, eps=1e-5):
    m = jnp.mean(x, axis=axis, keepdims=True)
    v = jnp.var(x, axis=axis, keepdims=True)
    return (x - m) / jnp.sqrt(v + eps)
def _scatter_add(tgt, idx, src, axis=0):
    return tgt.at[idx].add(src)
def _segment_sum(src, seg, n):
    return jax.ops.segment_sum(src, seg, n)
class _Rng:
    def __init__(self, key):
        self._k = key
    def _next(self):
        self._k, sub = jax.random.split(self._k)
        return sub
    def normal(self, shape):
        return jax.random.normal(self._next(), shape, dtype=jnp.bfloat16)
    def randint(self, lo, hi, shape):
        return jax.random.randint(self._next(), shape, lo, hi, dtype=jnp.int32)
    def uniform(self, shape, lo=0.0, hi=1.0):
        return jax.random.uniform(self._next(), shape, jnp.bfloat16, lo, hi)
    def permutation(self, n):
        return jax.random.permutation(self._next(), n)


kernel_name = 'gated_mix__compressed_kv_cla__sliding_block_cached__decode'

def setup_inputs():
    _rng = _Rng(jax.random.key(int.from_bytes(__import__("os").urandom(4), "little")))
    _w = (lambda a: (lambda t: t.astype(jnp.bfloat16) if jnp.issubdtype(t.dtype, jnp.floating) else t)(jnp.asarray(a)))
    def _A_setup():
        B, H, Sq, Sk, D, M = 8, 32, 1, 4096, 128, 512
        Dc = 4 * D
        return {
            "x": _w((lambda *s: _rng.normal(s) * 0.05)(B, Sq, M)),
            "c_kv": _w((lambda *s: _rng.normal(s) * 0.05)(B, Sk, Dc)),
            "w_q": _w((lambda *s: _rng.normal(s) * 0.05)(M, H, D) * (M ** -0.5)),
            "w_uk": _w((lambda *s: _rng.normal(s) * 0.05)(Dc, H, D) * (Dc ** -0.5)),
            "w_uv": _w((lambda *s: _rng.normal(s) * 0.05)(Dc, H, D) * (Dc ** -0.5)),
            "w_o": _w((lambda *s: _rng.normal(s) * 0.05)(H, D, M) * ((H * D) ** -0.5)),
        }
    _A_in = _A_setup()

    def _B_setup():
        B, Sq, D = 8, 1, 512
        Hq, Hkv, Sk, Dh = 32, 8, 4096, 128
        assert Hq % Hkv == 0, (Hq, Hkv)
        return {
            "x": _w((lambda *s: _rng.normal(s) * 0.05)(B, Sq, D)),
            "k_cache": _w((lambda *s: _rng.normal(s) * 0.05)(B, Hkv, Sk, Dh)),
            "v_cache": _w((lambda *s: _rng.normal(s) * 0.05)(B, Hkv, Sk, Dh)),
            "wq": _w((lambda *s: _rng.normal(s) * 0.05)(D, Hq * Dh) * (D ** -0.5)),
            "wo": _w((lambda *s: _rng.normal(s) * 0.05)(Hq * Dh, D) * ((Hq * Dh) ** -0.5)),
        }
    _B_in = _B_setup()

    return {
        "A_x": _A_in["x"],
        "A_c_kv": _A_in["c_kv"],
        "A_w_q": _A_in["w_q"],
        "A_w_uk": _A_in["w_uk"],
        "A_w_uv": _A_in["w_uv"],
        "A_w_o": _A_in["w_o"],
        "B_x": _B_in["x"],
        "B_k_cache": _B_in["k_cache"],
        "B_v_cache": _B_in["v_cache"],
        "B_wq": _B_in["wq"],
        "B_wo": _B_in["wo"],
        "gate_w": _w((lambda *s: _rng.normal(s) * 0.05)(512)),
    }

def reference(A_x, A_c_kv, A_w_q, A_w_uk, A_w_uv, A_w_o, B_x, B_k_cache, B_v_cache, B_wq, B_wo, gate_w):
    def _A_ref(x, c_kv, w_q, w_uk, w_uv, w_o):
        B, Sq, M = x.shape[0], x.shape[1], x.shape[2]
        Sk = c_kv.shape[1]
        H, D = w_q.shape[1], w_q.shape[2]
        q = jnp.einsum("bqm,mhd->bhqd", x, w_q)
        k = jnp.einsum("bkc,chd->bhkd", c_kv, w_uk)
        v = jnp.einsum("bkc,chd->bhkd", c_kv, w_uv)
        scores = jnp.einsum("bhqd,bhkd->bhqk", q, k) * (D ** -0.5)
        off = Sk - Sq
        qi = jnp.arange(Sq)[:, None]
        kj = jnp.arange(Sk)[None, :]
        cmask = kj <= (qi + off)
        scores = jnp.where(cmask[None, None], scores, -1e9)
        p = _softmax(scores, axis=-1)
        ctx = jnp.einsum("bhqk,bhkd->bhqd", p, v)
        return jnp.einsum("bhqd,hdm->bqm", ctx, w_o)

    def _B_ref(x, k_cache, v_cache, wq, wo):
        B, Sq, D = x.shape
        Hq, Dh = 32, 128
        Hkv, Sk = k_cache.shape[1], k_cache.shape[2]
        W = min(4096, max(256, Sk // 4))
        rep = Hq // Hkv
        q = (lambda x, *d: x.transpose(*d))((x @ wq).reshape(B, Sq, Hq, Dh), 0, 2, 1, 3)
        k = jnp.repeat(k_cache[:, :, Sk - W:, :], rep, axis=1)
        v = jnp.repeat(v_cache[:, :, Sk - W:, :], rep, axis=1)
        scores = jnp.einsum("bhqd,bhkd->bhqk", q, k) * (Dh ** -0.5)
        p = _softmax(scores, axis=-1)
        o = jnp.einsum("bhqk,bhkd->bhqd", p, v)
        return (lambda x, *d: x.transpose(*d))(o, 0, 2, 1, 3).reshape(B, Sq, Hq * Dh) @ wo

    x = A_x
    g = _sigmoid((x * gate_w).sum(-1, keepdims=True))
    a = _A_ref(x, A_c_kv, A_w_q, A_w_uk, A_w_uv, A_w_o)
    b = _B_ref(x, B_k_cache, B_v_cache, B_wq, B_wo)
    return g * a + (1 - g) * b
```

```python
import functools

import jax
import jax.numpy as jnp
from jax import lax
import jax.experimental.pallas as pl
import jax.experimental.pallas.tpu as pltpu

_LOG2E = 1.4426950408889634

_NB = 3
_CCH = 1024
_NWO = 4
_NBWO = 8

_NT = (((1,), (1,)), ((), ()))


def _dot(a, b):
    return jnp.dot(a, b, preferred_element_type=jnp.float32)


def _dot_nt(a, b):
    return lax.dot_general(a, b, _NT, preferred_element_type=jnp.float32)


def _kernel(
    x_hbm, c_hbm, wq_hbm, wuk_hbm, wuv_hbm, wo_hbm, k_hbm, v_hbm, bwq_hbm, bwo_hbm, gw_hbm,
    o_ref,
    x_v, gw_v, wq_v, wuk_v, wuv_v, wo_v, bwq_v, bwo_v, c_v, k_v, v_v,
    qa_s, ql_s, qb_s, cl_s, ob_s, ctx_s,
    sem_c, sem_k, sem_v, sem_w, sem_wo, sem_bwo,
    *, B, H, D, M, Sk, Dc, Hkv, W,
):
    REP = H // Hkv
    NCH = Sk // _CCH
    CT = Dc // 128
    HP = H // 2
    WO_H = H // _NWO
    BWO_H = H // _NBWO

    def c_copy(b, k):
        slot = b % _NB
        return pltpu.make_async_copy(
            c_hbm.at[b, pl.ds(k * _CCH, _CCH), :],
            c_v.at[slot, pl.ds(k * _CCH, _CCH), :],
            sem_c.at[slot, k])

    def k_copy(b):
        slot = b % _NB
        return pltpu.make_async_copy(
            k_hbm.at[b, :, pl.ds(Sk - W, W), :], k_v.at[slot], sem_k.at[slot])

    def v_copy(b):
        slot = b % _NB
        return pltpu.make_async_copy(
            v_hbm.at[b, :, pl.ds(Sk - W, W), :], v_v.at[slot], sem_v.at[slot])

    def in_order(n, start_fn):
        def body(i, carry):
            start_fn(i)
            return carry
        lax.fori_loop(0, n, body, 0)

    def in_order_list(thunks):
        def start_fn(i):
            for k, th in enumerate(thunks):
                pl.when(i == k)(th)
        in_order(len(thunks), start_fn)

    def start_batch(b):
        in_order(NCH, lambda k: c_copy(b, k).start())
        in_order_list([lambda: k_copy(b).start(), lambda: v_copy(b).start()])

    x_copy = pltpu.make_async_copy(x_hbm, x_v, sem_w.at[0])
    gw_copy = pltpu.make_async_copy(gw_hbm, gw_v, sem_w.at[1])
    wq_copy = pltpu.make_async_copy(wq_hbm.bitcast(jnp.uint32), wq_v, sem_w.at[2])
    wuk_copy = pltpu.make_async_copy(wuk_hbm.bitcast(jnp.uint32), wuk_v, sem_w.at[3])
    bwq_copy = pltpu.make_async_copy(bwq_hbm, bwq_v, sem_w.at[4])
    wuv_copy = pltpu.make_async_copy(wuv_hbm.bitcast(jnp.uint32), wuv_v, sem_w.at[5])

    def wo_copy(i):
        return pltpu.make_async_copy(
            wo_hbm.at[pl.ds(i * WO_H, WO_H)], wo_v.at[pl.ds(i * WO_H, WO_H)], sem_wo.at[i])

    def bwo_copy(i):
        rows = BWO_H * D
        return pltpu.make_async_copy(
            bwo_hbm.at[pl.ds(i * rows, rows)], bwo_v.at[pl.ds(i * rows, rows)], sem_bwo.at[i])

    def start_out_weights():
        in_order(1, lambda i: wuv_copy.start())
        in_order(_NWO, lambda i: wo_copy(i).start())
        in_order(_NBWO, lambda i: bwo_copy(i).start())

    def first_copies():
        x_copy.start()
        gw_copy.start()
        wq_copy.start()
    in_order_list([first_copies, wuk_copy.start, bwq_copy.start])
    in_order(_NB - 1, start_batch)

    def head_pair(w32, j):
        n = w32.shape[0] // H
        a = w32[pl.ds(j, n, stride=H), :]
        b_ = w32[pl.ds(HP + j, n, stride=H), :]
        even = (a & jnp.uint32(0xFFFF)) | (b_ << 16)
        odd = (a >> 16) | (b_ & jnp.uint32(0xFFFF0000))
        return pltpu.bitcast(even, jnp.bfloat16), pltpu.bitcast(odd, jnp.bfloat16)

    x_copy.wait()
    gw_copy.wait()
    x = x_v[...]
    gate_logit = jnp.sum(x.astype(jnp.float32) * gw_v[...].astype(jnp.float32).reshape(1, M),
                         axis=-1, keepdims=True)
    gate = jax.nn.sigmoid(gate_logit)

    wq_copy.wait()

    def qa_body(j, carry):
        we, wo_ = head_pair(wq_v, j)
        qa_s[pl.ds(pl.multiple_of(2 * j * B, B), B), :] = _dot(x, we)
        qa_s[pl.ds(pl.multiple_of((2 * j + 1) * B, B), B), :] = _dot(x, wo_)
        return carry
    lax.fori_loop(0, HP, qa_body, 0)

    wuk_copy.wait()
    scale_a = (D ** -0.5) * _LOG2E

    def ql_body(j, carry):
        we, wo_ = head_pair(wuk_v, j)
        for r, w in ((0, we), (1, wo_)):
            row = pl.multiple_of((2 * j + r) * B, B)
            q = qa_s[pl.ds(row, B), :].astype(jnp.bfloat16)
            ql = _dot_nt(q, w) * scale_a
            for t in range(CT):
                ql_s[t, pl.ds(row, B), :] = ql[:, t * 128:(t + 1) * 128]
        return carry
    lax.fori_loop(0, HP, ql_body, 0)

    bwq_copy.wait()
    scale_b = (D ** -0.5) * _LOG2E

    def qb_body(j, carry):
        w = bwq_v[:, pl.ds(pl.multiple_of(j * 4 * D, 4 * D), 4 * D)]
        q = _dot(x, w) * scale_b
        for i in range(4):
            qb_s[pl.ds(pl.multiple_of((4 * j + i) * B, B), B), :] = q[:, i * D:(i + 1) * D]
        return carry
    lax.fori_loop(0, H // 4, qb_body, 0)

    def batch_body(b, carry):
        slot = b % _NB

        @pl.when(b + _NB - 1 < B)
        def _():
            start_batch(b + _NB - 1)

        @pl.when(b + _NB - 1 == B)
        def _():
            start_out_weights()

        q = jnp.concatenate(
            [ql_s[t, pl.ds(b, H, stride=B), :] for t in range(CT)], axis=-1
        ).astype(jnp.bfloat16)

        def chunk_body(k, mla):
            m_prev, l_prev, acc = mla
            c_copy(b, k).wait()
            c = c_v[slot, pl.ds(pl.multiple_of(k * _CCH, _CCH), _CCH), :]
            s = _dot_nt(q, c)
            m_new = jnp.maximum(m_prev, jnp.max(s, axis=-1, keepdims=True))
            alpha = jnp.exp2(m_prev - m_new)
            p = jnp.exp2(s - m_new)
            l_new = alpha * l_prev + jnp.sum(p, axis=-1, keepdims=True)
            acc = alpha * acc + _dot(p.astype(jnp.bfloat16), c)
            return m_new, l_new, acc

        m0 = jnp.full((H, 1), -jnp.inf, jnp.float32)
        l0 = jnp.zeros((H, 1), jnp.float32)
        a0 = jnp.zeros((H, Dc), jnp.float32)
        _, l, acc = lax.fori_loop(0, NCH, chunk_body, (m0, l0, a0))
        cl = acc / l
        for t in range(CT):
            cl_s[t, pl.ds(pl.multiple_of(b * H, H), H), :] = cl[:, t * 128:(t + 1) * 128]

        k_copy(b).wait()
        v_copy(b).wait()
        first = lax.broadcasted_iota(jnp.int32, (2 * REP, 1), 0) < REP

        def pair_body(j, carry2):
            q8 = qb_s[pl.ds(j * 2 * REP * B + b, 2 * REP, stride=B), :].astype(jnp.bfloat16)
            s = jnp.where(first, _dot_nt(q8, k_v[slot, 2 * j]), _dot_nt(q8, k_v[slot, 2 * j + 1]))
            m = jnp.max(s, axis=-1, keepdims=True)
            p = jnp.exp2(s - m)
            lb = jnp.sum(p, axis=-1, keepdims=True)
            pb = p.astype(jnp.bfloat16)
            o = jnp.where(first, _dot(pb, v_v[slot, 2 * j]), _dot(pb, v_v[slot, 2 * j + 1]))
            ob_s[pl.ds(pl.multiple_of(b * H + j * 2 * REP, 2 * REP), 2 * REP), :] = o / lb
            return carry2
        lax.fori_loop(0, Hkv // 2, pair_body, 0)
        return carry

    lax.fori_loop(0, B, batch_body, 0)

    wuv_copy.wait()

    def ctx_body(j, carry):
        we, wo_ = head_pair(wuv_v, j)
        for r, w in ((0, we), (1, wo_)):
            h = 2 * j + r
            lhs = jnp.concatenate(
                [cl_s[t, pl.ds(h, B, stride=H), :] for t in range(CT)], axis=-1
            ).astype(jnp.bfloat16)
            ctx_s[pl.ds(pl.multiple_of(h * B, B), B), :] = _dot(lhs, w)
        return carry
    lax.fori_loop(0, HP, ctx_body, 0)

    out_a = jnp.zeros((B, M), jnp.float32)
    for i in range(_NWO):
        wo_copy(i).wait()

        def oa_body(hh, acc, i=i):
            h = i * WO_H + hh
            lhs = ctx_s[pl.ds(pl.multiple_of(h * B, B), B), :].astype(jnp.bfloat16)
            return acc + _dot(lhs, wo_v[h])
        out_a = lax.fori_loop(0, WO_H, oa_body, out_a)

    out_b = jnp.zeros((B, M), jnp.float32)
    for i in range(_NBWO):
        bwo_copy(i).wait()

        def ob_body(hh, acc, i=i):
            h = i * BWO_H + hh
            lhs = ob_s[pl.ds(h, B, stride=H), :].astype(jnp.bfloat16)
            return acc + _dot(lhs, bwo_v[pl.ds(pl.multiple_of(h * D, D), D), :])
        out_b = lax.fori_loop(0, BWO_H, ob_body, out_b)

    out = gate * out_a + (1.0 - gate) * out_b
    o_ref[...] = out.astype(o_ref.dtype)


@jax.jit
def pallas_gated_mix__compressed_kv_cla__sliding_block_cached__decode_kernel(
    A_x: jax.Array,
    A_c_kv: jax.Array,
    A_w_q: jax.Array,
    A_w_uk: jax.Array,
    A_w_uv: jax.Array,
    A_w_o: jax.Array,
    B_x: jax.Array,
    B_k_cache: jax.Array,
    B_v_cache: jax.Array,
    B_wq: jax.Array,
    B_wo: jax.Array,
    gate_w: jax.Array,
):
    del B_x
    B, Sq, M = A_x.shape
    Sk, Dc = A_c_kv.shape[1], A_c_kv.shape[2]
    H, D = A_w_q.shape[1], A_w_q.shape[2]
    Hkv = B_k_cache.shape[1]
    W = min(4096, max(256, B_k_cache.shape[2] // 4))
    assert Sq == 1 and D == 128 and B == 8 and H == 32 and B_k_cache.shape[2] == Sk
    assert Sk % _CCH == 0 and Dc % 128 == 0 and (H // Hkv) * 2 == 8
    bf = jnp.bfloat16

    kern = functools.partial(_kernel, B=B, H=H, D=D, M=M, Sk=Sk, Dc=Dc, Hkv=Hkv, W=W)
    hbm = pl.BlockSpec(memory_space=pl.ANY)
    f32 = jnp.float32
    out = pl.pallas_call(
        kern,
        out_shape=jax.ShapeDtypeStruct((B, M), A_x.dtype),
        in_specs=[hbm] * 11,
        out_specs=pl.BlockSpec(memory_space=pltpu.VMEM),
        scratch_shapes=[
            pltpu.VMEM((B, M), bf),
            pltpu.VMEM((M,), bf),
            pltpu.VMEM((M * H // 2, D), jnp.uint32),
            pltpu.VMEM((Dc * H // 2, D), jnp.uint32),
            pltpu.VMEM((Dc * H // 2, D), jnp.uint32),
            pltpu.VMEM((H, D, M), bf),
            pltpu.VMEM((M, H * D), bf),
            pltpu.VMEM((H * D, M), bf),
            pltpu.VMEM((_NB, Sk, Dc), bf),
            pltpu.VMEM((_NB, Hkv, W, D), bf),
            pltpu.VMEM((_NB, Hkv, W, D), bf),
            pltpu.VMEM((H * B, D), f32),
            pltpu.VMEM((Dc // 128, H * B, 128), f32),
            pltpu.VMEM((H * B, D), f32),
            pltpu.VMEM((Dc // 128, B * H, 128), f32),
            pltpu.VMEM((B * H, D), f32),
            pltpu.VMEM((H * B, D), f32),
            pltpu.SemaphoreType.DMA((_NB, Sk // _CCH)),
            pltpu.SemaphoreType.DMA((_NB,)),
            pltpu.SemaphoreType.DMA((_NB,)),
            pltpu.SemaphoreType.DMA((6,)),
            pltpu.SemaphoreType.DMA((_NWO,)),
            pltpu.SemaphoreType.DMA((_NBWO,)),
        ],
        compiler_params=pltpu.CompilerParams(vmem_limit_bytes=96 * 2**20),
    )(
        A_x.reshape(B, M), A_c_kv,
        A_w_q.reshape(M * H, D), A_w_uk.reshape(Dc * H, D), A_w_uv.reshape(Dc * H, D),
        A_w_o, B_k_cache, B_v_cache, B_wq, B_wo, gate_w,
    )
    return out.reshape(B, Sq, M)
```

```python
import functools
import math

import jax
import jax.numpy as jnp
from jax import lax
import jax.experimental.pallas as pl
import jax.experimental.pallas.tpu as pltpu

_LOG2E = 1.4426950408889634

_NB = 3
_CCH = 1024
_NWO = 4
_BWO_PIECES = (8, 8, 8, 4, 2, 1, 1)
_TWO_QUEUES = True

_NT = (((1,), (1,)), ((), ()))


def _dot(a, b):
    return jnp.dot(a, b, preferred_element_type=jnp.float32)


def _dot_nt(a, b):
    return lax.dot_general(a, b, _NT, preferred_element_type=jnp.float32)


def _kernel(
    x_hbm, c_hbm, wq_hbm, wuk_hbm, wuv_hbm, wo_hbm, k_hbm, v_hbm, bwq_hbm, bwo_hbm, gw_hbm,
    o_ref,
    x_v, gw_v, wq_v, wuk_v, wuv_v, wo_v, bwq_v, bwo_v, c_v, k_v, v_v,
    qa_s, ql_s, qb_s, cl_s, ob_s, ctx_s,
    sem_c, sem_k, sem_v, sem_w, sem_wo, sem_bwo,
    *, B, H, D, M, Sk, Dc, Hkv, W,
):
    REP = H // Hkv
    NCH = Sk // _CCH
    CT = Dc // 128
    HP = H // 2
    WO_H = H // _NWO
    NPAIR = Hkv // 2

    def in_order(n, start_fn):
        def body(i, carry):
            start_fn(i)
            return carry
        lax.fori_loop(0, n, body, 0)

    class Transfer:
        def __init__(self, src, dst, sem):
            self.src, self.dst, self.sem = src, dst, sem

        def start(self, part=0, nparts=1, split=True):
            rows = self.src.shape[0] // nparts
            assert rows * nparts == self.src.shape[0]
            nq = 2 if (split and _TWO_QUEUES and rows % 2 == 0) else 1
            step = rows // nq
            for q in range(nq):
                rng = pl.ds(part * rows + q * step, step)
                pltpu.make_async_copy(self.src.at[rng], self.dst.at[rng], self.sem).start(priority=q)

        def wait(self):
            pltpu.make_async_copy(self.src, self.dst, self.sem).wait()

    def c_copy(b, k):
        slot, rng = b % _NB, pl.ds(k * _CCH, _CCH)
        return Transfer(c_hbm.at[b, rng], c_v.at[slot, rng], sem_c.at[slot, k])

    def k_copy(b, j):
        slot, rng = b % _NB, pl.ds(2 * j, 2)
        return pltpu.make_async_copy(
            k_hbm.at[b, rng, pl.ds(Sk - W, W)], k_v.at[slot, rng], sem_k.at[slot, j])

    def v_copy(b, j):
        slot, rng = b % _NB, pl.ds(2 * j, 2)
        return pltpu.make_async_copy(
            v_hbm.at[b, rng, pl.ds(Sk - W, W)], v_v.at[slot, rng], sem_v.at[slot, j])

    def start_c(b):
        in_order(NCH, lambda k: c_copy(b, k).start())

    def start_kv_pair(b, j):
        k_copy(b, j).start(priority=0)
        v_copy(b, j).start(priority=1 if _TWO_QUEUES else 0)

    def start_kv(b):
        in_order(NPAIR, lambda j: start_kv_pair(b, j))

    x_copy = Transfer(x_hbm, x_v, sem_w.at[0])
    gw_copy = Transfer(gw_hbm, gw_v, sem_w.at[1])
    wq_copy = Transfer(wq_hbm.bitcast(jnp.uint32), wq_v, sem_w.at[2])
    wuk_copy = Transfer(wuk_hbm.bitcast(jnp.uint32), wuk_v, sem_w.at[3])
    bwq_copy = Transfer(bwq_hbm, bwq_v, sem_w.at[4])
    wuv_copy = Transfer(wuv_hbm.bitcast(jnp.uint32), wuv_v, sem_w.at[5])

    def wo_copy(i):
        rng = pl.ds(i * WO_H * D, WO_H * D)
        return Transfer(wo_hbm.at[rng], wo_v.at[rng], sem_wo.at[i])

    bwo_start = [sum(_BWO_PIECES[:i]) for i in range(len(_BWO_PIECES))]

    def bwo_copy(i):
        rng = pl.ds(bwo_start[i] * D, _BWO_PIECES[i] * D)
        return Transfer(bwo_hbm.at[rng], bwo_v.at[rng], sem_bwo.at[i])

    wq_copy.start(split=False)
    x_copy.start(split=False)
    gw_copy.start(split=False)
    wuk_copy.start(split=False)

    def head_pair(w32, j):
        n = w32.shape[0] // H
        a = w32[pl.ds(j, n, stride=H), :]
        b_ = w32[pl.ds(HP + j, n, stride=H), :]
        even = (a & jnp.uint32(0xFFFF)) | (b_ << 16)
        odd = (a >> 16) | (b_ & jnp.uint32(0xFFFF0000))
        return pltpu.bitcast(even, jnp.bfloat16), pltpu.bitcast(odd, jnp.bfloat16)

    x_copy.wait()
    gw_copy.wait()
    x = x_v[...]
    gate_logit = jnp.sum(x.astype(jnp.float32) * gw_v[...].astype(jnp.float32).reshape(1, M),
                         axis=-1, keepdims=True)
    gate = jax.nn.sigmoid(gate_logit)

    wq_copy.wait()
    start_c(0)

    def qa_body(j, carry):
        we, wo_ = head_pair(wq_v, j)
        qa_s[pl.ds(pl.multiple_of(2 * j * B, B), B), :] = _dot(x, we)
        qa_s[pl.ds(pl.multiple_of((2 * j + 1) * B, B), B), :] = _dot(x, wo_)
        return carry
    lax.fori_loop(0, HP, qa_body, 0)

    wuk_copy.wait()
    start_c(1)
    scale_a = (D ** -0.5) * _LOG2E

    def ql_body(j, carry):
        we, wo_ = head_pair(wuk_v, j)
        for r, w in ((0, we), (1, wo_)):
            row = pl.multiple_of((2 * j + r) * B, B)
            q = qa_s[pl.ds(row, B), :].astype(jnp.bfloat16)
            ql = _dot_nt(q, w) * scale_a
            for t in range(CT):
                ql_s[t, pl.ds(row, B), :] = ql[:, t * 128:(t + 1) * 128]
        return carry
    lax.fori_loop(0, HP, ql_body, 0)

    def a_body(b, carry):
        slot = b % _NB

        q = jnp.concatenate(
            [ql_s[t, pl.ds(b, H, stride=B), :] for t in range(CT)], axis=-1
        ).astype(jnp.bfloat16)

        def chunk_body(k, mla):
            m_prev, l_prev, acc = mla
            c_copy(b, k).wait()

            @pl.when(b + 2 < B)
            def _():
                c_copy(b + 2, k).start()

            @pl.when(b + 2 == B)
            def _():
                wuv_copy.start(k, NCH)

            @pl.when(b + 2 == B + 1)
            def _():
                wo_copy(k).start()

            c = c_v[slot, pl.ds(pl.multiple_of(k * _CCH, _CCH), _CCH), :]
            s = _dot_nt(q, c)
            m_new = jnp.maximum(m_prev, jnp.max(s, axis=-1, keepdims=True))
            alpha = jnp.exp2(m_prev - m_new)
            p = jnp.exp2(s - m_new)
            l_new = alpha * l_prev + jnp.sum(p, axis=-1, keepdims=True)
            acc = alpha * acc + _dot(p.astype(jnp.bfloat16), c)
            return m_new, l_new, acc

        m0 = jnp.full((H, 1), -jnp.inf, jnp.float32)
        l0 = jnp.zeros((H, 1), jnp.float32)
        a0 = jnp.zeros((H, Dc), jnp.float32)
        _, l, acc = lax.fori_loop(0, NCH, chunk_body, (m0, l0, a0))
        cl = acc / l
        for t in range(CT):
            cl_s[t, pl.ds(pl.multiple_of(b * H, H), H), :] = cl[:, t * 128:(t + 1) * 128]
        return carry

    lax.fori_loop(0, B, a_body, 0)

    wuv_copy.wait()
    in_order(4, lambda i: bwq_copy.start(i, 4))

    def ctx_body(j, carry):
        we, wo_ = head_pair(wuv_v, j)
        for r, w in ((0, we), (1, wo_)):
            h = 2 * j + r
            lhs = jnp.concatenate(
                [cl_s[t, pl.ds(h, B, stride=H), :] for t in range(CT)], axis=-1
            ).astype(jnp.bfloat16)
            ctx_s[pl.ds(pl.multiple_of(h * B, B), B), :] = _dot(lhs, w)
        return carry
    lax.fori_loop(0, HP, ctx_body, 0)

    start_kv(0)

    def oa_body(i, acc):
        lhs = jnp.concatenate(
            [ctx_s[pl.ds(pl.multiple_of((i * WO_H + hh) * B, B), B), :] for hh in range(WO_H)],
            axis=-1).astype(jnp.bfloat16)
        wo_copy(i).wait()
        return acc + _dot(lhs, wo_v[pl.ds(pl.multiple_of(i * WO_H * D, WO_H * D), WO_H * D), :])
    out_a = lax.fori_loop(0, _NWO, oa_body, jnp.zeros((B, M), jnp.float32))
    out_a = gate * out_a

    bwq_copy.wait()
    start_kv(1)
    scale_b = (D ** -0.5) * _LOG2E

    def qb_body(j, carry):
        w = bwq_v[:, pl.ds(pl.multiple_of(j * 4 * D, 4 * D), 4 * D)]
        q = _dot(x, w) * scale_b
        for i in range(4):
            qb_s[pl.ds(pl.multiple_of((4 * j + i) * B, B), B), :] = q[:, i * D:(i + 1) * D]
        return carry
    lax.fori_loop(0, H // 4, qb_body, 0)

    first = lax.broadcasted_iota(jnp.int32, (2 * REP, 1), 0) < REP

    def b_body(b, carry):
        slot = b % _NB

        def pair_body(j, carry2):
            q8 = qb_s[pl.ds(j * 2 * REP * B + b, 2 * REP, stride=B), :].astype(jnp.bfloat16)
            k_copy(b, j).wait()

            @pl.when(b + 2 < B)
            def _():
                start_kv_pair(b + 2, j)

            for jj in range(NPAIR):
                @pl.when((b + 2 == B) & (j == jj))
                def _(jj=jj):
                    last = jj == NPAIR - 1
                    for i in range(jj, len(_BWO_PIECES) if last else jj + 1):
                        in_order(1, lambda _, i=i: bwo_copy(i).start())

            s = jnp.where(first, _dot_nt(q8, k_v[slot, 2 * j]), _dot_nt(q8, k_v[slot, 2 * j + 1]))
            m = jnp.max(s, axis=-1, keepdims=True)
            p = jnp.exp2(s - m)
            lb = jnp.sum(p, axis=-1, keepdims=True)
            pb = p.astype(jnp.bfloat16)
            v_copy(b, j).wait()
            o = jnp.where(first, _dot(pb, v_v[slot, 2 * j]), _dot(pb, v_v[slot, 2 * j + 1]))
            ob_s[pl.ds(pl.multiple_of(b * H + j * 2 * REP, 2 * REP), 2 * REP), :] = o / lb
            return carry2
        lax.fori_loop(0, NPAIR, pair_body, 0)
        return carry

    lax.fori_loop(0, B, b_body, 0)

    out_b = jnp.zeros((B, M), jnp.float32)
    for i, nh in enumerate(_BWO_PIECES):
        h0 = bwo_start[i]
        lhs = jnp.concatenate(
            [ob_s[pl.ds(h, B, stride=H), :] for h in range(h0, h0 + nh)], axis=-1
        ).astype(jnp.bfloat16)
        bwo_copy(i).wait()
        out_b = out_b + _dot(lhs, bwo_v[pl.ds(h0 * D, nh * D), :])

    o_ref[...] = (out_a + (1.0 - gate) * out_b).astype(o_ref.dtype)


@jax.jit
def pallas_gated_mix__compressed_kv_cla__sliding_block_cached__decode_kernel(
    A_x: jax.Array,
    A_c_kv: jax.Array,
    A_w_q: jax.Array,
    A_w_uk: jax.Array,
    A_w_uv: jax.Array,
    A_w_o: jax.Array,
    B_x: jax.Array,
    B_k_cache: jax.Array,
    B_v_cache: jax.Array,
    B_wq: jax.Array,
    B_wo: jax.Array,
    gate_w: jax.Array,
):
    del B_x
    B, Sq, M = A_x.shape
    Sk, Dc = A_c_kv.shape[1], A_c_kv.shape[2]
    H, D = A_w_q.shape[1], A_w_q.shape[2]
    Hkv = B_k_cache.shape[1]
    W = min(4096, max(256, B_k_cache.shape[2] // 4))
    assert Sq == 1 and D == 128 and B == 8 and H == 32 and B_k_cache.shape[2] == Sk
    assert sum(_BWO_PIECES) == H and _NB >= 3 and _NWO == Sk // _CCH
    assert Sk % _CCH == 0 and Dc % 128 == 0 and (H // Hkv) * 2 == 8
    bf = jnp.bfloat16

    kern = functools.partial(_kernel, B=B, H=H, D=D, M=M, Sk=Sk, Dc=Dc, Hkv=Hkv, W=W)
    hbm = pl.BlockSpec(memory_space=pl.ANY)
    f32 = jnp.float32
    out = pl.pallas_call(
        kern,
        out_shape=jax.ShapeDtypeStruct((B, M), A_x.dtype),
        in_specs=[hbm] * 11,
        out_specs=pl.BlockSpec(memory_space=pltpu.VMEM),
        scratch_shapes=[
            pltpu.VMEM((B, M), bf),
            pltpu.VMEM((M,), bf),
            pltpu.VMEM((M * H // 2, D), jnp.uint32),
            pltpu.VMEM((Dc * H // 2, D), jnp.uint32),
            pltpu.VMEM((Dc * H // 2, D), jnp.uint32),
            pltpu.VMEM((H * D, M), bf),
            pltpu.VMEM((M, H * D), bf),
            pltpu.VMEM((H * D, M), bf),
            pltpu.VMEM((_NB, Sk, Dc), bf),
            pltpu.VMEM((_NB, Hkv, W, D), bf),
            pltpu.VMEM((_NB, Hkv, W, D), bf),
            pltpu.VMEM((H * B, D), f32),
            pltpu.VMEM((Dc // 128, H * B, 128), f32),
            pltpu.VMEM((H * B, D), f32),
            pltpu.VMEM((Dc // 128, B * H, 128), f32),
            pltpu.VMEM((B * H, D), f32),
            pltpu.VMEM((H * B, D), f32),
            pltpu.SemaphoreType.DMA((_NB, Sk // _CCH)),
            pltpu.SemaphoreType.DMA((_NB, Hkv // 2)),
            pltpu.SemaphoreType.DMA((_NB, Hkv // 2)),
            pltpu.SemaphoreType.DMA((6,)),
            pltpu.SemaphoreType.DMA((_NWO,)),
            pltpu.SemaphoreType.DMA((len(_BWO_PIECES),)),
        ],
        compiler_params=pltpu.CompilerParams(vmem_limit_bytes=96 * 2**20),
    )(
        A_x.reshape(B, M), A_c_kv,
        A_w_q.reshape(M * H, D), A_w_uk.reshape(Dc * H, D), A_w_uv.reshape(Dc * H, D),
        A_w_o.reshape(H * D, M), B_k_cache, B_v_cache, B_wq, B_wo, gate_w,
    )
    return out.reshape(B, Sq, M)
```

```python
import functools

import jax
import jax.numpy as jnp
from jax import lax
import jax.experimental.pallas as pl
import jax.experimental.pallas.tpu as pltpu

_LOG2E = 1.4426950408889634
_NCH = 4
_NB = 3
_NQ = 2
_TAIL = (4, 2, 1, 1)

_NT = (((1,), (1,)), ((), ()))


def _dot(a, b):
    return jnp.dot(a, b, preferred_element_type=jnp.float32)


def _dot_nt(a, b):
    return lax.dot_general(a, b, _NT, preferred_element_type=jnp.float32)


def _kernel(
    x_hbm, c_hbm, wq_hbm, wuk_hbm, wuv_hbm, wo_hbm, k_hbm, v_hbm, bwq_hbm, bwo_hbm, gw_hbm,
    o_ref,
    x_v, gw_v, wq_v, wuk_v, wuv_v, wo_v, bwq_v, bwo_v, c_v, k_v, v_v,
    qa_s, ql_s, qb_s, cl_s, ob_s, ctx_s,
    sem_c, sem_k, sem_v, sem_w, sem_x, sem_tail,
    *, B, H, D, M, Sk, Dc, Hkv, W,
):
    f32, bf16 = jnp.float32, jnp.bfloat16
    REP = H // Hkv
    CCH = Sk // _NCH
    CT = Dc // 128
    HP = H // 2
    HC = H // _NCH

    class Chunk:
        def __init__(self, src, dst, sem):
            self.src, self.dst, self.sem = src, dst, sem

        def start(self, nq=_NQ):
            step = self.src.shape[0] // nq
            for q in range(nq):
                rng = pl.ds(q * step, step)
                pltpu.make_async_copy(
                    self.src.at[rng], self.dst.at[rng], self.sem).start(priority=q)

        def wait(self):
            pltpu.make_async_copy(self.src, self.dst, self.sem).wait()

    def rows_chunk(hbm, vmem, k, sem):
        n = hbm.shape[0] // _NCH
        rng = pl.ds(pl.multiple_of(k * n, n), n)
        return Chunk(hbm.at[rng], vmem.at[rng], sem)

    def wq_chunk(k): return rows_chunk(wq_hbm, wq_v, k, sem_w.at[0, k])
    def wuk_chunk(k): return rows_chunk(wuk_hbm, wuk_v, k, sem_w.at[1, k])
    def wuv_chunk(k): return rows_chunk(wuv_hbm, wuv_v, k, sem_w.at[2, k])
    def wo_chunk(k): return rows_chunk(wo_hbm, wo_v, k, sem_w.at[3, k])
    def bwq_chunk(k): return rows_chunk(bwq_hbm, bwq_v, k, sem_w.at[4, k])
    def bwo_chunk(k): return rows_chunk(bwo_hbm, bwo_v, k, sem_w.at[5, k])

    def c_chunk(b, k):
        return rows_chunk(c_hbm.at[b], c_v.at[b % _NB], k, sem_c.at[b % _NB, k])

    def k_chunk(b, j):
        rng = pl.ds(2 * j, 2)
        return pltpu.make_async_copy(k_hbm.at[b, rng, pl.ds(Sk - W, W)],
                                     k_v.at[b % _NB, rng], sem_k.at[b % _NB, j])

    def v_chunk(b, j):
        rng = pl.ds(2 * j, 2)
        return pltpu.make_async_copy(v_hbm.at[b, rng, pl.ds(Sk - W, W)],
                                     v_v.at[b % _NB, rng], sem_v.at[b % _NB, j])

    def start_kv(b, j):
        k_chunk(b, j).start(priority=0)
        v_chunk(b, j).start(priority=_NQ - 1)

    tail_h0 = [H - HC + sum(_TAIL[:i]) for i in range(len(_TAIL))]

    def bwo_tail(i):
        rng = pl.ds(tail_h0[i] * D, _TAIL[i] * D)
        return Chunk(bwo_hbm.at[rng], bwo_v.at[rng], sem_tail.at[i])

    def in_order(n, start_fn):
        def body(i, carry):
            start_fn(i)
            return carry
        lax.fori_loop(0, n, body, 0)

    x_copy = Chunk(x_hbm, x_v, sem_x.at[0])
    gw_copy = Chunk(gw_hbm, gw_v, sem_x.at[1])
    in_order(_NCH, lambda k: wq_chunk(k).start(nq=1))
    x_copy.start(nq=1)
    gw_copy.start(nq=1)
    in_order(_NCH, lambda k: wuk_chunk(k).start(nq=1))

    def head_pairs(w_v, k):
        n = w_v.shape[0] // _NCH
        w = w_v[pl.ds(pl.multiple_of(k * n, n), n), :]
        u = pltpu.bitcast(w, jnp.uint32).reshape(n // H, HP, D)
        u = jnp.swapaxes(u, 0, 1)
        for p in range(HP):
            even = pltpu.bitcast(u[p] << 16, f32).astype(bf16)
            odd = pltpu.bitcast(u[p] & jnp.uint32(0xFFFF0000), f32).astype(bf16)
            yield 2 * p, even
            yield 2 * p + 1, odd

    def head_rows(h):
        return pl.ds(h * B, B)

    x_copy.wait()
    gw_copy.wait()

    qa_s[...] = jnp.zeros_like(qa_s)

    def qa_body(k, carry):
        wq_chunk(k).wait()
        c_chunk(0, k).start()
        xk = x_v[:, pl.ds(pl.multiple_of(k * 128, 128), 128)]
        for h, w in head_pairs(wq_v, k):
            qa_s[head_rows(h), :] += _dot(xk, w)
        return carry
    lax.fori_loop(0, _NCH, qa_body, 0)

    scale = (D ** -0.5) * _LOG2E

    def ql_body(k, carry):
        wuk_chunk(k).wait()
        c_chunk(1, k).start()
        for h, w in head_pairs(wuk_v, k):
            q = qa_s[head_rows(h), :].astype(bf16)
            ql_s[k, head_rows(h), :] = _dot_nt(q, w) * scale
        return carry
    lax.fori_loop(0, _NCH, ql_body, 0)

    def a_body(b, carry):
        q = jnp.concatenate(
            [ql_s[t, pl.ds(b, H, stride=B), :] for t in range(CT)], axis=-1
        ).astype(bf16)

        def chunk_body(k, mla):
            m_prev, l_prev, acc = mla
            c_chunk(b, k).wait()

            @pl.when(b + 2 < B)
            def _():
                c_chunk(b + 2, k).start()

            @pl.when(b + 2 == B)
            def _():
                wuv_chunk(k).start()

            @pl.when(b + 2 == B + 1)
            def _():
                wo_chunk(k).start()

            c = c_v[b % _NB, pl.ds(pl.multiple_of(k * CCH, CCH), CCH), :]
            s = _dot_nt(q, c)
            m_new = jnp.maximum(m_prev, jnp.max(s, axis=-1, keepdims=True))
            alpha = jnp.exp2(m_prev - m_new)
            p = jnp.exp2(s - m_new)
            l_new = alpha * l_prev + jnp.sum(p, axis=-1, keepdims=True)
            acc = alpha * acc + _dot(p.astype(bf16), c)
            return m_new, l_new, acc

        m0 = jnp.full((H, 1), -jnp.inf, f32)
        l0 = jnp.zeros((H, 1), f32)
        a0 = jnp.zeros((H, Dc), f32)
        _, l, acc = lax.fori_loop(0, _NCH, chunk_body, (m0, l0, a0))
        cl = acc / l
        for t in range(CT):
            cl_s[t, pl.ds(pl.multiple_of(b * H, H), H), :] = cl[:, t * 128:(t + 1) * 128]
        return carry

    lax.fori_loop(0, B, a_body, 0)

    ctx_s[...] = jnp.zeros_like(ctx_s)

    def ctx_body(k, carry):
        wuv_chunk(k).wait()
        bwq_chunk(k).start()
        for h, w in head_pairs(wuv_v, k):
            lhs = cl_s[k, pl.ds(h, B, stride=H), :].astype(bf16)
            ctx_s[head_rows(h), :] += _dot(lhs, w)
        return carry
    lax.fori_loop(0, _NCH, ctx_body, 0)

    def out_proj(lhs_heads, w_v, k, acc):
        lhs = jnp.concatenate(lhs_heads, axis=-1).astype(bf16)
        n = w_v.shape[0] // _NCH
        return acc + _dot(lhs, w_v[pl.ds(pl.multiple_of(k * n, n), n), :])

    def oa_body(k, acc):
        wo_chunk(k).wait()
        start_kv(0, k)
        lhs = [ctx_s[pl.ds(pl.multiple_of((k * HC + i) * B, B), B), :] for i in range(HC)]
        return out_proj(lhs, wo_v, k, acc)
    out_a = lax.fori_loop(0, _NCH, oa_body, jnp.zeros((B, M), f32))

    gate_logit = jnp.sum(x_v[...].astype(f32) * gw_v[...].astype(f32).reshape(1, M),
                         axis=-1, keepdims=True)
    gate = jax.nn.sigmoid(gate_logit)
    out_a = gate * out_a

    qb_s[...] = jnp.zeros_like(qb_s)

    def qb_body(k, carry):
        bwq_chunk(k).wait()
        start_kv(1, k)
        xk = x_v[:, pl.ds(pl.multiple_of(k * 128, 128), 128)]
        q = _dot(xk, bwq_v[pl.ds(pl.multiple_of(k * 128, 128), 128), :]) * scale
        for h in range(H):
            qb_s[head_rows(h), :] += q[:, h * D:(h + 1) * D]
        return carry
    lax.fori_loop(0, _NCH, qb_body, 0)

    first = lax.broadcasted_iota(jnp.int32, (2 * REP, 1), 0) < REP

    def b_body(b, carry):
        def pair_body(j, carry2):
            q8 = qb_s[pl.ds(j * 2 * REP * B + b, 2 * REP, stride=B), :].astype(bf16)
            k_chunk(b, j).wait()

            @pl.when(b + 2 < B)
            def _():
                start_kv(b + 2, j)

            @pl.when((b + 2 == B) & (j < _NCH - 1))
            def _():
                bwo_chunk(j).start()

            @pl.when((b + 2 == B) & (j == _NCH - 1))
            def _():
                for i in range(len(_TAIL)):
                    in_order(1, lambda _, i=i: bwo_tail(i).start())

            kk, vv = k_v.at[b % _NB], v_v.at[b % _NB]
            s = jnp.where(first, _dot_nt(q8, kk[2 * j]), _dot_nt(q8, kk[2 * j + 1]))
            m = jnp.max(s, axis=-1, keepdims=True)
            p = jnp.exp2(s - m)
            lb = jnp.sum(p, axis=-1, keepdims=True)
            pb = p.astype(bf16)
            v_chunk(b, j).wait()
            o = jnp.where(first, _dot(pb, vv[2 * j]), _dot(pb, vv[2 * j + 1]))
            ob_s[pl.ds(pl.multiple_of(b * H + j * 2 * REP, 2 * REP), 2 * REP), :] = o / lb
            return carry2
        lax.fori_loop(0, _NCH, pair_body, 0)
        return carry

    lax.fori_loop(0, B, b_body, 0)

    def ob_heads(h0, n):
        return [ob_s[pl.ds(h0 + i, B, stride=H), :] for i in range(n)]

    def ob_body(k, acc):
        bwo_chunk(k).wait()
        return out_proj(ob_heads(k * HC, HC), bwo_v, k, acc)
    out_b = lax.fori_loop(0, _NCH - 1, ob_body, jnp.zeros((B, M), f32))
    for i, n in enumerate(_TAIL):
        lhs = jnp.concatenate(ob_heads(tail_h0[i], n), axis=-1).astype(bf16)
        bwo_tail(i).wait()
        out_b = out_b + _dot(lhs, bwo_v[pl.ds(tail_h0[i] * D, n * D), :])

    o_ref[...] = (out_a + (1.0 - gate) * out_b).astype(o_ref.dtype)


@jax.jit
def pallas_gated_mix__compressed_kv_cla__sliding_block_cached__decode_kernel(
    A_x: jax.Array,
    A_c_kv: jax.Array,
    A_w_q: jax.Array,
    A_w_uk: jax.Array,
    A_w_uv: jax.Array,
    A_w_o: jax.Array,
    B_x: jax.Array,
    B_k_cache: jax.Array,
    B_v_cache: jax.Array,
    B_wq: jax.Array,
    B_wo: jax.Array,
    gate_w: jax.Array,
):
    del B_x
    B, Sq, M = A_x.shape
    Sk, Dc = A_c_kv.shape[1], A_c_kv.shape[2]
    H, D = A_w_q.shape[1], A_w_q.shape[2]
    Hkv, Skb = B_k_cache.shape[1], B_k_cache.shape[2]
    W = min(4096, max(256, Skb // 4))
    assert Sq == 1 and B == 8 and D == 128 and Skb == Sk
    assert M == _NCH * 128 and Dc == _NCH * 128 and Hkv == 2 * _NCH and H == 4 * Hkv
    assert sum(_TAIL) == H // _NCH and _NB >= 3
    bf, f32 = jnp.bfloat16, jnp.float32

    kern = functools.partial(_kernel, B=B, H=H, D=D, M=M, Sk=Sk, Dc=Dc, Hkv=Hkv, W=W)
    out = pl.pallas_call(
        kern,
        out_shape=jax.ShapeDtypeStruct((B, M), A_x.dtype),
        in_specs=[pl.BlockSpec(memory_space=pl.ANY)] * 11,
        out_specs=pl.BlockSpec(memory_space=pltpu.VMEM),
        scratch_shapes=[
            pltpu.VMEM((B, M), bf),
            pltpu.VMEM((M,), bf),
            pltpu.VMEM((M * H, D), bf),
            pltpu.VMEM((Dc * H, D), bf),
            pltpu.VMEM((Dc * H, D), bf),
            pltpu.VMEM((H * D, M), bf),
            pltpu.VMEM((M, H * D), bf),
            pltpu.VMEM((H * D, M), bf),
            pltpu.VMEM((_NB, Sk, Dc), bf),
            pltpu.VMEM((_NB, Hkv, W, D), bf),
            pltpu.VMEM((_NB, Hkv, W, D), bf),
            pltpu.VMEM((H * B, D), f32),
            pltpu.VMEM((Dc // 128, H * B, 128), f32),
            pltpu.VMEM((H * B, D), f32),
            pltpu.VMEM((Dc // 128, B * H, 128), f32),
            pltpu.VMEM((B * H, D), f32),
            pltpu.VMEM((H * B, D), f32),
            pltpu.SemaphoreType.DMA((_NB, _NCH)),
            pltpu.SemaphoreType.DMA((_NB, _NCH)),
            pltpu.SemaphoreType.DMA((_NB, _NCH)),
            pltpu.SemaphoreType.DMA((6, _NCH)),
            pltpu.SemaphoreType.DMA((2,)),
            pltpu.SemaphoreType.DMA((len(_TAIL),)),
        ],
        compiler_params=pltpu.CompilerParams(vmem_limit_bytes=80 * 2**20),
    )(
        A_x.reshape(B, M), A_c_kv,
        A_w_q.reshape(M * H, D), A_w_uk.reshape(Dc * H, D), A_w_uv.reshape(Dc * H, D),
        A_w_o.reshape(H * D, M), B_k_cache, B_v_cache, B_wq, B_wo, gate_w,
    )
    return out.reshape(B, Sq, M)
```

```python
import functools

import jax
import jax.numpy as jnp
from jax import lax
import jax.experimental.pallas as pl
import jax.experimental.pallas.tpu as pltpu

_LOG2E = 1.4426950408889634
_NCH = 4
_NB = 3
_TAIL = (4, 2, 2)

_NT = (((1,), (1,)), ((), ()))


def _dot(a, b):
    return jnp.dot(a, b, preferred_element_type=jnp.float32)


def _dot_nt(a, b):
    return lax.dot_general(a, b, _NT, preferred_element_type=jnp.float32)


def _kernel(
    x_hbm, c_hbm, wq_hbm, wuk_hbm, wuv_hbm, wo_hbm, k_hbm, v_hbm, bwq_hbm, bwo_hbm, gw_hbm,
    o_ref,
    x_v, gw_v, wq_v, wuk_v, wuv_v, wo_v, bwq_v, bwo_v, c_v, k_v, v_v,
    qa_s, ql_s, qb_s, cl_s, ob_s, ctx_s,
    sems, tail_sems,
    *, B, H, D, M, Sk, Dc, Hkv, W,
):
    f32, bf16 = jnp.float32, jnp.bfloat16
    REP = H // Hkv
    CCH = Sk // _NCH
    CT = Dc // 128
    HP = H // 2
    HC = H // _NCH

    class Chunk:
        def __init__(self, sem, *pairs):
            self.sem, self.pairs = sem, pairs

        def start(self):
            for src, dst in self.pairs:
                step = src.shape[0] // 2
                for q in range(2):
                    rng = pl.ds(q * step, step)
                    pltpu.make_async_copy(src.at[rng], dst.at[rng], self.sem).start(priority=q)

        def wait(self):
            for src, dst in self.pairs:
                pltpu.make_async_copy(src, dst, self.sem).wait()

    def rows_chunk(hbm, vmem, item, k):
        n = hbm.shape[0] // _NCH
        rng = pl.ds(pl.multiple_of(k * n, n), n)
        return Chunk(sems.at[item % 2, k], (hbm.at[rng], vmem.at[rng]))

    def wq_chunk(k): return rows_chunk(wq_hbm, wq_v, 0, k)
    def wuk_chunk(k): return rows_chunk(wuk_hbm, wuk_v, 1, k)
    def c_chunk(b, k): return rows_chunk(c_hbm.at[b], c_v.at[b % _NB], 2 + b, k)
    def wuv_chunk(k): return rows_chunk(wuv_hbm, wuv_v, 2 + B, k)
    def wo_chunk(k): return rows_chunk(wo_hbm, wo_v, 3 + B, k)
    def bwq_chunk(k): return rows_chunk(bwq_hbm, bwq_v, 4 + B, k)
    def bwo_chunk(k): return rows_chunk(bwo_hbm, bwo_v, 5 + 2 * B, k)

    def kv_chunk(b, j):
        rng, win = pl.ds(2 * j, 2), pl.ds(Sk - W, W)
        return Chunk(sems.at[(5 + B + b) % 2, j],
                     (k_hbm.at[b, rng, win], k_v.at[b % _NB, rng]),
                     (v_hbm.at[b, rng, win], v_v.at[b % _NB, rng]))

    tail_h0 = [H - HC + sum(_TAIL[:i]) for i in range(len(_TAIL))]

    def bwo_tail(i):
        rng = pl.ds(tail_h0[i] * D, _TAIL[i] * D)
        sem = sems.at[(5 + 2 * B) % 2, _NCH - 1] if i == 0 else tail_sems.at[i - 1]
        return Chunk(sem, (bwo_hbm.at[rng], bwo_v.at[rng]))

    def in_order(n, start_fn):
        def body(i, carry):
            start_fn(i)
            return carry
        lax.fori_loop(0, n, body, 0)

    x_copy = pltpu.make_async_copy(x_hbm, x_v, tail_sems.at[0])
    gw_copy = pltpu.make_async_copy(gw_hbm, gw_v, tail_sems.at[1])
    x_copy.start()
    gw_copy.start()
    in_order(_NCH, lambda k: wq_chunk(k).start())
    in_order(_NCH, lambda k: wuk_chunk(k).start())

    def head_pairs(w_v, k):
        n = w_v.shape[0] // _NCH
        w = w_v[pl.ds(pl.multiple_of(k * n, n), n), :]
        u = pltpu.bitcast(w, jnp.uint32).reshape(n // H, HP, D)
        u = jnp.swapaxes(u, 0, 1)
        for p in range(HP):
            even = pltpu.bitcast(u[p] << 16, f32).astype(bf16)
            odd = pltpu.bitcast(u[p] & jnp.uint32(0xFFFF0000), f32).astype(bf16)
            yield 2 * p, even
            yield 2 * p + 1, odd

    def head_rows(h):
        return pl.ds(h * B, B)

    x_copy.wait()
    gw_copy.wait()

    qa_s[...] = jnp.zeros_like(qa_s)

    def qa_body(k, carry):
        wq_chunk(k).wait()
        c_chunk(0, k).start()
        xk = x_v[:, pl.ds(pl.multiple_of(k * 128, 128), 128)]
        for h, w in head_pairs(wq_v, k):
            qa_s[head_rows(h), :] += _dot(xk, w)
        return carry
    lax.fori_loop(0, _NCH, qa_body, 0)

    scale = (D ** -0.5) * _LOG2E

    def ql_body(k, carry):
        wuk_chunk(k).wait()
        c_chunk(1, k).start()
        for h, w in head_pairs(wuk_v, k):
            q = qa_s[head_rows(h), :].astype(bf16)
            ql_s[k, head_rows(h), :] = _dot_nt(q, w) * scale
        return carry
    lax.fori_loop(0, _NCH, ql_body, 0)

    def a_body(b, carry):
        q = jnp.concatenate(
            [ql_s[t, pl.ds(b, H, stride=B), :] for t in range(CT)], axis=-1
        ).astype(bf16)

        def chunk_body(k, mla):
            m_prev, l_prev, acc = mla
            c_chunk(b, k).wait()

            @pl.when(b + 2 < B)
            def _():
                c_chunk(b + 2, k).start()

            @pl.when(b + 2 == B)
            def _():
                wuv_chunk(k).start()

            @pl.when(b + 2 == B + 1)
            def _():
                wo_chunk(k).start()

            c = c_v[b % _NB, pl.ds(pl.multiple_of(k * CCH, CCH), CCH), :]
            s = _dot_nt(q, c)
            m_new = jnp.maximum(m_prev, jnp.max(s, axis=-1, keepdims=True))
            alpha = jnp.exp2(m_prev - m_new)
            p = jnp.exp2(s - m_new)
            l_new = alpha * l_prev + jnp.sum(p, axis=-1, keepdims=True)
            acc = alpha * acc + _dot(p.astype(bf16), c)
            return m_new, l_new, acc

        m0 = jnp.full((H, 1), -jnp.inf, f32)
        l0 = jnp.zeros((H, 1), f32)
        a0 = jnp.zeros((H, Dc), f32)
        _, l, acc = lax.fori_loop(0, _NCH, chunk_body, (m0, l0, a0))
        cl = acc / l
        for t in range(CT):
            cl_s[t, pl.ds(pl.multiple_of(b * H, H), H), :] = cl[:, t * 128:(t + 1) * 128]
        return carry

    lax.fori_loop(0, B, a_body, 0)

    ctx_s[...] = jnp.zeros_like(ctx_s)

    def ctx_body(k, carry):
        wuv_chunk(k).wait()
        bwq_chunk(k).start()
        for h, w in head_pairs(wuv_v, k):
            lhs = cl_s[k, pl.ds(h, B, stride=H), :].astype(bf16)
            ctx_s[head_rows(h), :] += _dot(lhs, w)
        return carry
    lax.fori_loop(0, _NCH, ctx_body, 0)

    def out_proj(lhs_heads, w_v, k, acc):
        lhs = jnp.concatenate(lhs_heads, axis=-1).astype(bf16)
        n = w_v.shape[0] // _NCH
        return acc + _dot(lhs, w_v[pl.ds(pl.multiple_of(k * n, n), n), :])

    def oa_body(k, acc):
        wo_chunk(k).wait()
        kv_chunk(0, k).start()
        lhs = [ctx_s[pl.ds(pl.multiple_of((k * HC + i) * B, B), B), :] for i in range(HC)]
        return out_proj(lhs, wo_v, k, acc)
    out_a = lax.fori_loop(0, _NCH, oa_body, jnp.zeros((B, M), f32))

    gate_logit = jnp.sum(x_v[...].astype(f32) * gw_v[...].astype(f32).reshape(1, M),
                         axis=-1, keepdims=True)
    gate = jax.nn.sigmoid(gate_logit)
    out_a = gate * out_a

    qb_s[...] = jnp.zeros_like(qb_s)

    def qb_body(k, carry):
        bwq_chunk(k).wait()
        kv_chunk(1, k).start()
        xk = x_v[:, pl.ds(pl.multiple_of(k * 128, 128), 128)]
        q = _dot(xk, bwq_v[pl.ds(pl.multiple_of(k * 128, 128), 128), :]) * scale
        for h in range(H):
            qb_s[head_rows(h), :] += q[:, h * D:(h + 1) * D]
        return carry
    lax.fori_loop(0, _NCH, qb_body, 0)

    first = lax.broadcasted_iota(jnp.int32, (2 * REP, 1), 0) < REP

    def b_body(b, carry):
        def pair_body(j, carry2):
            q8 = qb_s[pl.ds(j * 2 * REP * B + b, 2 * REP, stride=B), :].astype(bf16)
            kv_chunk(b, j).wait()

            @pl.when(b + 2 < B)
            def _():
                kv_chunk(b + 2, j).start()

            @pl.when((b + 2 == B) & (j < _NCH - 1))
            def _():
                bwo_chunk(j).start()

            @pl.when((b + 2 == B) & (j == _NCH - 1))
            def _():
                for i in range(len(_TAIL)):
                    in_order(1, lambda _, i=i: bwo_tail(i).start())

            kk, vv = k_v.at[b % _NB], v_v.at[b % _NB]
            s = jnp.where(first, _dot_nt(q8, kk[2 * j]), _dot_nt(q8, kk[2 * j + 1]))
            m = jnp.max(s, axis=-1, keepdims=True)
            p = jnp.exp2(s - m)
            lb = jnp.sum(p, axis=-1, keepdims=True)
            pb = p.astype(bf16)
            o = jnp.where(first, _dot(pb, vv[2 * j]), _dot(pb, vv[2 * j + 1]))
            ob_s[pl.ds(pl.multiple_of(b * H + j * 2 * REP, 2 * REP), 2 * REP), :] = o / lb
            return carry2
        lax.fori_loop(0, _NCH, pair_body, 0)
        return carry

    lax.fori_loop(0, B, b_body, 0)

    def ob_heads(h0, n):
        return [ob_s[pl.ds(h0 + i, B, stride=H), :] for i in range(n)]

    def ob_body(k, acc):
        bwo_chunk(k).wait()
        return out_proj(ob_heads(k * HC, HC), bwo_v, k, acc)
    out_b = lax.fori_loop(0, _NCH - 1, ob_body, jnp.zeros((B, M), f32))
    for i, n in enumerate(_TAIL):
        lhs = jnp.concatenate(ob_heads(tail_h0[i], n), axis=-1).astype(bf16)
        bwo_tail(i).wait()
        out_b = out_b + _dot(lhs, bwo_v[pl.ds(tail_h0[i] * D, n * D), :])

    o_ref[...] = (out_a + (1.0 - gate) * out_b).astype(o_ref.dtype)


@jax.jit
def pallas_gated_mix__compressed_kv_cla__sliding_block_cached__decode_kernel(
    A_x: jax.Array,
    A_c_kv: jax.Array,
    A_w_q: jax.Array,
    A_w_uk: jax.Array,
    A_w_uv: jax.Array,
    A_w_o: jax.Array,
    B_x: jax.Array,
    B_k_cache: jax.Array,
    B_v_cache: jax.Array,
    B_wq: jax.Array,
    B_wo: jax.Array,
    gate_w: jax.Array,
):
    del B_x
    B, Sq, M = A_x.shape
    Sk, Dc = A_c_kv.shape[1], A_c_kv.shape[2]
    H, D = A_w_q.shape[1], A_w_q.shape[2]
    Hkv, Skb = B_k_cache.shape[1], B_k_cache.shape[2]
    W = min(4096, max(256, Skb // 4))
    assert Sq == 1 and B == 8 and D == 128 and Skb == Sk
    assert M == _NCH * 128 and Dc == _NCH * 128 and Hkv == 2 * _NCH and H == 4 * Hkv
    assert sum(_TAIL) == H // _NCH and len(_TAIL) >= 3 and _NB >= 3
    bf, f32 = jnp.bfloat16, jnp.float32

    kern = functools.partial(_kernel, B=B, H=H, D=D, M=M, Sk=Sk, Dc=Dc, Hkv=Hkv, W=W)
    out = pl.pallas_call(
        kern,
        out_shape=jax.ShapeDtypeStruct((B, M), A_x.dtype),
        in_specs=[pl.BlockSpec(memory_space=pl.ANY)] * 11,
        out_specs=pl.BlockSpec(memory_space=pltpu.VMEM),
        scratch_shapes=[
            pltpu.VMEM((B, M), bf),
            pltpu.VMEM((M,), bf),
            pltpu.VMEM((M * H, D), bf),
            pltpu.VMEM((Dc * H, D), bf),
            pltpu.VMEM((Dc * H, D), bf),
            pltpu.VMEM((H * D, M), bf),
            pltpu.VMEM((M, H * D), bf),
            pltpu.VMEM((H * D, M), bf),
            pltpu.VMEM((_NB, Sk, Dc), bf),
            pltpu.VMEM((_NB, Hkv, W, D), bf),
            pltpu.VMEM((_NB, Hkv, W, D), bf),
            pltpu.VMEM((H * B, D), f32),
            pltpu.VMEM((Dc // 128, H * B, 128), f32),
            pltpu.VMEM((H * B, D), f32),
            pltpu.VMEM((Dc // 128, B * H, 128), f32),
            pltpu.VMEM((B * H, D), f32),
            pltpu.VMEM((H * B, D), f32),
            pltpu.SemaphoreType.DMA((2, _NCH)),
            pltpu.SemaphoreType.DMA((len(_TAIL) - 1,)),
        ],
        compiler_params=pltpu.CompilerParams(vmem_limit_bytes=80 * 2**20),
    )(
        A_x.reshape(B, M), A_c_kv,
        A_w_q.reshape(M * H, D), A_w_uk.reshape(Dc * H, D), A_w_uv.reshape(Dc * H, D),
        A_w_o.reshape(H * D, M), B_k_cache, B_v_cache, B_wq, B_wo, gate_w,
    )
    return out.reshape(B, Sq, M)
```

```python
import functools

import jax
import jax.numpy as jnp
from jax import lax
import jax.experimental.pallas as pl
import jax.experimental.pallas.tpu as pltpu

_LOG2E = 1.4426950408889634
_NCH = 4
_NB = 2
_TAIL = (4, 2, 2)

_NT = (((1,), (1,)), ((), ()))


def _dot(a, b):
    return jnp.dot(a, b, preferred_element_type=jnp.float32)


def _dot_nt(a, b):
    return lax.dot_general(a, b, _NT, preferred_element_type=jnp.float32)


def _kernel(
    x_hbm, c_hbm, wq_hbm, wuk_hbm, wuv_hbm, wo_hbm, k_hbm, v_hbm, bwq_hbm, bwo_hbm, gw_hbm,
    o_ref,
    x_v, gw_v, wq_v, wuk_v, wuv_v, wo_v, bwq_v, bwo_v, c_v, k_v, v_v,
    qa_s, ql_s, qb_s, cl_s, ob_s, ctx_s,
    sems, tail_sems,
    *, B, H, D, M, Sk, Dc, Hkv, W,
):
    f32, bf16 = jnp.float32, jnp.bfloat16
    REP = H // Hkv
    CCH = Sk // _NCH
    CT = Dc // 128
    HP = H // 2
    HC = H // _NCH

    class Chunk:
        def __init__(self, sem, *pairs):
            self.sem, self.pairs = sem, pairs

        def start(self):
            for src, dst in self.pairs:
                step = src.shape[0] // 2
                for q in range(2):
                    rng = pl.ds(q * step, step)
                    pltpu.make_async_copy(src.at[rng], dst.at[rng], self.sem).start(priority=q)

        def wait(self):
            for src, dst in self.pairs:
                pltpu.make_async_copy(src, dst, self.sem).wait()

    def rows_chunk(hbm, vmem, k):
        n = hbm.shape[0] // _NCH
        rng = pl.ds(pl.multiple_of(k * n, n), n)
        return Chunk(sems.at[k], (hbm.at[rng], vmem.at[rng]))

    def wq_chunk(k): return rows_chunk(wq_hbm, wq_v, k)
    def wuk_chunk(k): return rows_chunk(wuk_hbm, wuk_v, k)
    def c_chunk(b, k): return rows_chunk(c_hbm.at[b], c_v.at[b % _NB], k)
    def wuv_chunk(k): return rows_chunk(wuv_hbm, wuv_v, k)
    def wo_chunk(k): return rows_chunk(wo_hbm, wo_v, k)
    def bwq_chunk(k): return rows_chunk(bwq_hbm, bwq_v, k)
    def bwo_chunk(k): return rows_chunk(bwo_hbm, bwo_v, k)

    def kv_chunk(b, j):
        rng, win = pl.ds(2 * j, 2), pl.ds(Sk - W, W)
        return Chunk(sems.at[j],
                     (k_hbm.at[b, rng, win], k_v.at[b % _NB, rng]),
                     (v_hbm.at[b, rng, win], v_v.at[b % _NB, rng]))

    tail_h0 = [H - HC + sum(_TAIL[:i]) for i in range(len(_TAIL))]

    def bwo_tail(i):
        rng = pl.ds(tail_h0[i] * D, _TAIL[i] * D)
        sem = sems.at[_NCH - 1] if i == 0 else tail_sems.at[i - 1]
        return Chunk(sem, (bwo_hbm.at[rng], bwo_v.at[rng]))

    def in_order(n, start_fn):
        def body(i, carry):
            start_fn(i)
            return carry
        lax.fori_loop(0, n, body, 0)

    x_copy = pltpu.make_async_copy(x_hbm, x_v, tail_sems.at[0])
    gw_copy = pltpu.make_async_copy(gw_hbm, gw_v, tail_sems.at[1])
    x_copy.start()
    gw_copy.start()
    in_order(_NCH, lambda k: wq_chunk(k).start())

    def head_pairs(w_v, k):
        n = w_v.shape[0] // _NCH
        w = w_v[pl.ds(pl.multiple_of(k * n, n), n), :]
        u = pltpu.bitcast(w, jnp.uint32).reshape(n // H, HP, D)
        u = jnp.swapaxes(u, 0, 1)
        for p in range(HP):
            even = pltpu.bitcast(u[p] << 16, f32).astype(bf16)
            odd = pltpu.bitcast(u[p] & jnp.uint32(0xFFFF0000), f32).astype(bf16)
            yield 2 * p, even
            yield 2 * p + 1, odd

    def head_rows(h):
        return pl.ds(h * B, B)

    x_copy.wait()
    gw_copy.wait()

    qa_s[...] = jnp.zeros_like(qa_s)

    def qa_body(k, carry):
        wq_chunk(k).wait()
        wuk_chunk(k).start()
        xk = x_v[:, pl.ds(pl.multiple_of(k * 128, 128), 128)]
        for h, w in head_pairs(wq_v, k):
            qa_s[head_rows(h), :] += _dot(xk, w)
        return carry
    lax.fori_loop(0, _NCH, qa_body, 0)

    scale = (D ** -0.5) * _LOG2E

    def ql_body(k, carry):
        wuk_chunk(k).wait()
        c_chunk(0, k).start()
        for h, w in head_pairs(wuk_v, k):
            q = qa_s[head_rows(h), :].astype(bf16)
            ql_s[k, head_rows(h), :] = _dot_nt(q, w) * scale
        return carry
    lax.fori_loop(0, _NCH, ql_body, 0)

    def a_body(b, carry):
        q = jnp.concatenate(
            [ql_s[t, pl.ds(b, H, stride=B), :] for t in range(CT)], axis=-1
        ).astype(bf16)

        def chunk_body(k, mla):
            m_prev, l_prev, acc = mla
            c_chunk(b, k).wait()

            @pl.when(b + 1 < B)
            def _():
                c_chunk(b + 1, k).start()

            @pl.when(b + 1 == B)
            def _():
                wuv_chunk(k).start()

            c = c_v[b % _NB, pl.ds(pl.multiple_of(k * CCH, CCH), CCH), :]
            s = _dot_nt(q, c)
            m_new = jnp.maximum(m_prev, jnp.max(s, axis=-1, keepdims=True))
            alpha = jnp.exp2(m_prev - m_new)
            p = jnp.exp2(s - m_new)
            l_new = alpha * l_prev + jnp.sum(p, axis=-1, keepdims=True)
            acc = alpha * acc + _dot(p.astype(bf16), c)
            return m_new, l_new, acc

        m0 = jnp.full((H, 1), -jnp.inf, f32)
        l0 = jnp.zeros((H, 1), f32)
        a0 = jnp.zeros((H, Dc), f32)
        _, l, acc = lax.fori_loop(0, _NCH, chunk_body, (m0, l0, a0))
        cl = acc / l
        for t in range(CT):
            cl_s[t, pl.ds(pl.multiple_of(b * H, H), H), :] = cl[:, t * 128:(t + 1) * 128]
        return carry

    lax.fori_loop(0, B, a_body, 0)

    ctx_s[...] = jnp.zeros_like(ctx_s)

    def ctx_body(k, carry):
        wuv_chunk(k).wait()
        wo_chunk(k).start()
        for h, w in head_pairs(wuv_v, k):
            lhs = cl_s[k, pl.ds(h, B, stride=H), :].astype(bf16)
            ctx_s[head_rows(h), :] += _dot(lhs, w)
        return carry
    lax.fori_loop(0, _NCH, ctx_body, 0)

    def out_proj(lhs_heads, w_v, k, acc):
        lhs = jnp.concatenate(lhs_heads, axis=-1).astype(bf16)
        n = w_v.shape[0] // _NCH
        return acc + _dot(lhs, w_v[pl.ds(pl.multiple_of(k * n, n), n), :])

    def oa_body(k, acc):
        wo_chunk(k).wait()
        bwq_chunk(k).start()
        lhs = [ctx_s[pl.ds(pl.multiple_of((k * HC + i) * B, B), B), :] for i in range(HC)]
        return out_proj(lhs, wo_v, k, acc)
    out_a = lax.fori_loop(0, _NCH, oa_body, jnp.zeros((B, M), f32))

    gate_logit = jnp.sum(x_v[...].astype(f32) * gw_v[...].astype(f32).reshape(1, M),
                         axis=-1, keepdims=True)
    gate = jax.nn.sigmoid(gate_logit)
    out_a = gate * out_a

    qb_s[...] = jnp.zeros_like(qb_s)

    def qb_body(k, carry):
        bwq_chunk(k).wait()
        kv_chunk(0, k).start()
        xk = x_v[:, pl.ds(pl.multiple_of(k * 128, 128), 128)]
        q = _dot(xk, bwq_v[pl.ds(pl.multiple_of(k * 128, 128), 128), :]) * scale
        for h in range(H):
            qb_s[head_rows(h), :] += q[:, h * D:(h + 1) * D]
        return carry
    lax.fori_loop(0, _NCH, qb_body, 0)

    first = lax.broadcasted_iota(jnp.int32, (2 * REP, 1), 0) < REP

    def b_body(b, carry):
        def pair_body(j, carry2):
            q8 = qb_s[pl.ds(j * 2 * REP * B + b, 2 * REP, stride=B), :].astype(bf16)
            kv_chunk(b, j).wait()

            @pl.when(b + 1 < B)
            def _():
                kv_chunk(b + 1, j).start()

            @pl.when((b + 1 == B) & (j < _NCH - 1))
            def _():
                bwo_chunk(j).start()

            @pl.when((b + 1 == B) & (j == _NCH - 1))
            def _():
                for i in range(len(_TAIL)):
                    in_order(1, lambda _, i=i: bwo_tail(i).start())

            kk, vv = k_v.at[b % _NB], v_v.at[b % _NB]
            s = jnp.where(first, _dot_nt(q8, kk[2 * j]), _dot_nt(q8, kk[2 * j + 1]))
            m = jnp.max(s, axis=-1, keepdims=True)
            p = jnp.exp2(s - m)
            lb = jnp.sum(p, axis=-1, keepdims=True)
            pb = p.astype(bf16)
            o = jnp.where(first, _dot(pb, vv[2 * j]), _dot(pb, vv[2 * j + 1]))
            ob_s[pl.ds(pl.multiple_of(b * H + j * 2 * REP, 2 * REP), 2 * REP), :] = o / lb
            return carry2
        lax.fori_loop(0, _NCH, pair_body, 0)
        return carry

    lax.fori_loop(0, B, b_body, 0)

    def ob_heads(h0, n):
        return [ob_s[pl.ds(h0 + i, B, stride=H), :] for i in range(n)]

    def ob_body(k, acc):
        bwo_chunk(k).wait()
        return out_proj(ob_heads(k * HC, HC), bwo_v, k, acc)
    out_b = lax.fori_loop(0, _NCH - 1, ob_body, jnp.zeros((B, M), f32))
    for i, n in enumerate(_TAIL):
        lhs = jnp.concatenate(ob_heads(tail_h0[i], n), axis=-1).astype(bf16)
        bwo_tail(i).wait()
        out_b = out_b + _dot(lhs, bwo_v[pl.ds(tail_h0[i] * D, n * D), :])

    o_ref[...] = (out_a + (1.0 - gate) * out_b).astype(o_ref.dtype)


@jax.jit
def pallas_gated_mix__compressed_kv_cla__sliding_block_cached__decode_kernel(
    A_x: jax.Array,
    A_c_kv: jax.Array,
    A_w_q: jax.Array,
    A_w_uk: jax.Array,
    A_w_uv: jax.Array,
    A_w_o: jax.Array,
    B_x: jax.Array,
    B_k_cache: jax.Array,
    B_v_cache: jax.Array,
    B_wq: jax.Array,
    B_wo: jax.Array,
    gate_w: jax.Array,
):
    del B_x
    B, Sq, M = A_x.shape
    Sk, Dc = A_c_kv.shape[1], A_c_kv.shape[2]
    H, D = A_w_q.shape[1], A_w_q.shape[2]
    Hkv, Skb = B_k_cache.shape[1], B_k_cache.shape[2]
    W = min(4096, max(256, Skb // 4))
    assert Sq == 1 and B == 8 and D == 128 and Skb == Sk
    assert M == _NCH * 128 and Dc == _NCH * 128 and Hkv == 2 * _NCH and H == 4 * Hkv
    assert sum(_TAIL) == H // _NCH and len(_TAIL) >= 3 and _NB >= 2
    bf, f32 = jnp.bfloat16, jnp.float32

    kern = functools.partial(_kernel, B=B, H=H, D=D, M=M, Sk=Sk, Dc=Dc, Hkv=Hkv, W=W)
    out = pl.pallas_call(
        kern,
        out_shape=jax.ShapeDtypeStruct((B, M), A_x.dtype),
        in_specs=[pl.BlockSpec(memory_space=pl.ANY)] * 11,
        out_specs=pl.BlockSpec(memory_space=pltpu.VMEM),
        scratch_shapes=[
            pltpu.VMEM((B, M), bf),
            pltpu.VMEM((M,), bf),
            pltpu.VMEM((M * H, D), bf),
            pltpu.VMEM((Dc * H, D), bf),
            pltpu.VMEM((Dc * H, D), bf),
            pltpu.VMEM((H * D, M), bf),
            pltpu.VMEM((M, H * D), bf),
            pltpu.VMEM((H * D, M), bf),
            pltpu.VMEM((_NB, Sk, Dc), bf),
            pltpu.VMEM((_NB, Hkv, W, D), bf),
            pltpu.VMEM((_NB, Hkv, W, D), bf),
            pltpu.VMEM((H * B, D), f32),
            pltpu.VMEM((Dc // 128, H * B, 128), f32),
            pltpu.VMEM((H * B, D), f32),
            pltpu.VMEM((Dc // 128, B * H, 128), f32),
            pltpu.VMEM((B * H, D), f32),
            pltpu.VMEM((H * B, D), f32),
            pltpu.SemaphoreType.DMA((_NCH,)),
            pltpu.SemaphoreType.DMA((len(_TAIL) - 1,)),
        ],
        compiler_params=pltpu.CompilerParams(vmem_limit_bytes=80 * 2**20),
    )(
        A_x.reshape(B, M), A_c_kv,
        A_w_q.reshape(M * H, D), A_w_uk.reshape(Dc * H, D), A_w_uv.reshape(Dc * H, D),
        A_w_o.reshape(H * D, M), B_k_cache, B_v_cache, B_wq, B_wo, gate_w,
    )
    return out.reshape(B, Sq, M)
```

```python
import functools

import jax
import jax.numpy as jnp
from jax import lax
import jax.experimental.pallas as pl
import jax.experimental.pallas.tpu as pltpu

_LOG2E = 1.4426950408889634
_NCH = 4
_NB = 2
_TAIL = (4, 2, 2)

_NT = (((1,), (1,)), ((), ()))


def _dot(a, b):
    return jnp.dot(a, b, preferred_element_type=jnp.float32)


def _dot_nt(a, b):
    return lax.dot_general(a, b, _NT, preferred_element_type=jnp.float32)


def _kernel(
    x_hbm, c_hbm, wq_hbm, wuk_hbm, wuv_hbm, wo_hbm, k_hbm, v_hbm, bwq_hbm, bwo_hbm, gw_hbm,
    o_ref,
    x_v, gw_v, wq_v, wuk_v, wuv_v, wo_v, bwq_v, bwo_v, c_v, k_v, v_v,
    qa_s, ql_s, qb_s, cl_s, ob_s, ctx_s,
    sems, tail_sems,
    *, B, H, D, M, Sk, Dc, Hkv, W,
):
    f32, bf16 = jnp.float32, jnp.bfloat16
    REP = H // Hkv
    CCH = Sk // _NCH
    CT = Dc // 128
    HP = H // 2
    HC = H // _NCH

    class Chunk:
        def __init__(self, sem, *pairs):
            self.copies = []
            for src, dst in pairs:
                step = src.shape[0] // 2
                for q in range(2):
                    rng = pl.ds(q * step, step)
                    self.copies.append((pltpu.make_async_copy(src.at[rng], dst.at[rng], sem), q))

        def start(self):
            for copy, queue in self.copies:
                copy.start(priority=queue)

        def wait(self):
            for copy, _ in self.copies:
                copy.wait()

    def rows_chunk(hbm, vmem, k):
        n = hbm.shape[0] // _NCH
        rng = pl.ds(pl.multiple_of(k * n, n), n)
        return Chunk(sems.at[k], (hbm.at[rng], vmem.at[rng]))

    def wq_chunk(k): return rows_chunk(wq_hbm, wq_v, k)
    def wuk_chunk(k): return rows_chunk(wuk_hbm, wuk_v, k)
    def c_chunk(b, k): return rows_chunk(c_hbm.at[b], c_v.at[b % _NB], k)
    def wuv_chunk(k): return rows_chunk(wuv_hbm, wuv_v, k)
    def wo_chunk(k): return rows_chunk(wo_hbm, wo_v, k)
    def bwq_chunk(k): return rows_chunk(bwq_hbm, bwq_v, k)
    def bwo_chunk(k): return rows_chunk(bwo_hbm, bwo_v, k)

    def kv_chunk(b, j):
        rng, win = pl.ds(2 * j, 2), pl.ds(Sk - W, W)
        return Chunk(sems.at[j],
                     (k_hbm.at[b, rng, win], k_v.at[b % _NB, rng]),
                     (v_hbm.at[b, rng, win], v_v.at[b % _NB, rng]))

    tail_h0 = [H - HC + sum(_TAIL[:i]) for i in range(len(_TAIL))]

    def bwo_tail(i):
        rng = pl.ds(tail_h0[i] * D, _TAIL[i] * D)
        sem = sems.at[_NCH - 1] if i == 0 else tail_sems.at[i - 1]
        return Chunk(sem, (bwo_hbm.at[rng], bwo_v.at[rng]))

    def in_order(n, start_fn):
        def body(i, carry):
            start_fn(i)
            return carry
        lax.fori_loop(0, n, body, 0)

    x_copy = pltpu.make_async_copy(x_hbm, x_v, tail_sems.at[0])
    gw_copy = pltpu.make_async_copy(gw_hbm, gw_v, tail_sems.at[1])
    x_copy.start()
    gw_copy.start()
    in_order(_NCH, lambda k: wq_chunk(k).start())

    def head_pairs(w_v, k):
        n = w_v.shape[0] // _NCH
        w = w_v[pl.ds(pl.multiple_of(k * n, n), n), :]
        u = pltpu.bitcast(w, jnp.uint32).reshape(n // H, HP, D)
        u = jnp.swapaxes(u, 0, 1)
        for p in range(HP):
            even = pltpu.bitcast(u[p] << 16, f32).astype(bf16)
            odd = pltpu.bitcast(u[p] & jnp.uint32(0xFFFF0000), f32).astype(bf16)
            yield 2 * p, even
            yield 2 * p + 1, odd

    def head_rows(h):
        return pl.ds(h * B, B)

    x_copy.wait()
    gw_copy.wait()

    qa_s[...] = jnp.zeros_like(qa_s)

    def qa_body(k, carry):
        wq_chunk(k).wait()
        wuk_chunk(k).start()
        xk = x_v[:, pl.ds(pl.multiple_of(k * 128, 128), 128)]
        for h, w in head_pairs(wq_v, k):
            qa_s[head_rows(h), :] += _dot(xk, w)
        return carry
    lax.fori_loop(0, _NCH, qa_body, 0)

    scale = (D ** -0.5) * _LOG2E

    def ql_body(k, carry):
        wuk_chunk(k).wait()
        c_chunk(0, k).start()
        for h, w in head_pairs(wuk_v, k):
            q = qa_s[head_rows(h), :].astype(bf16)
            ql_s[k, head_rows(h), :] = _dot_nt(q, w) * scale
        return carry
    lax.fori_loop(0, _NCH, ql_body, 0)

    def a_body(b, carry):
        q = jnp.concatenate(
            [ql_s[t, pl.ds(b, H, stride=B), :] for t in range(CT)], axis=-1
        ).astype(bf16)

        def chunk_body(k, mla):
            m_prev, l_prev, acc = mla
            c_chunk(b, k).wait()

            @pl.when(b + 1 < B)
            def _():
                c_chunk(b + 1, k).start()

            @pl.when(b + 1 == B)
            def _():
                wuv_chunk(k).start()

            c = c_v[b % _NB, pl.ds(pl.multiple_of(k * CCH, CCH), CCH), :]
            s = _dot_nt(q, c)
            m_new = jnp.maximum(m_prev, jnp.max(s, axis=-1, keepdims=True))
            alpha = jnp.exp2(m_prev - m_new)
            p = jnp.exp2(s - m_new)
            l_new = alpha * l_prev + jnp.sum(p, axis=-1, keepdims=True)
            acc = alpha * acc + _dot(p.astype(bf16), c)
            return m_new, l_new, acc

        m0 = jnp.full((H, 1), -jnp.inf, f32)
        l0 = jnp.zeros((H, 1), f32)
        a0 = jnp.zeros((H, Dc), f32)
        _, l, acc = lax.fori_loop(0, _NCH, chunk_body, (m0, l0, a0))
        cl = acc / l
        for t in range(CT):
            cl_s[t, pl.ds(pl.multiple_of(b * H, H), H), :] = cl[:, t * 128:(t + 1) * 128]
        return carry

    lax.fori_loop(0, B, a_body, 0)

    ctx_s[...] = jnp.zeros_like(ctx_s)

    def ctx_body(k, carry):
        wuv_chunk(k).wait()
        wo_chunk(k).start()
        for h, w in head_pairs(wuv_v, k):
            lhs = cl_s[k, pl.ds(h, B, stride=H), :].astype(bf16)
            ctx_s[head_rows(h), :] += _dot(lhs, w)
        return carry
    lax.fori_loop(0, _NCH, ctx_body, 0)

    def out_proj(lhs_heads, w_v, k, acc):
        lhs = jnp.concatenate(lhs_heads, axis=-1).astype(bf16)
        n = w_v.shape[0] // _NCH
        return acc + _dot(lhs, w_v[pl.ds(pl.multiple_of(k * n, n), n), :])

    def oa_body(k, acc):
        wo_chunk(k).wait()
        bwq_chunk(k).start()
        lhs = [ctx_s[pl.ds(pl.multiple_of((k * HC + i) * B, B), B), :] for i in range(HC)]
        return out_proj(lhs, wo_v, k, acc)
    out_a = lax.fori_loop(0, _NCH, oa_body, jnp.zeros((B, M), f32))

    gate_logit = jnp.sum(x_v[...].astype(f32) * gw_v[...].astype(f32).reshape(1, M),
                         axis=-1, keepdims=True)
    gate = jax.nn.sigmoid(gate_logit)
    out_a = gate * out_a

    qb_s[...] = jnp.zeros_like(qb_s)

    def qb_body(k, carry):
        bwq_chunk(k).wait()
        kv_chunk(0, k).start()
        xk = x_v[:, pl.ds(pl.multiple_of(k * 128, 128), 128)]
        q = _dot(xk, bwq_v[pl.ds(pl.multiple_of(k * 128, 128), 128), :]) * scale
        for h in range(H):
            qb_s[head_rows(h), :] += q[:, h * D:(h + 1) * D]
        return carry
    lax.fori_loop(0, _NCH, qb_body, 0)

    first = lax.broadcasted_iota(jnp.int32, (2 * REP, 1), 0) < REP

    def b_body(b, carry):
        def pair_body(j, carry2):
            q8 = qb_s[pl.ds(j * 2 * REP * B + b, 2 * REP, stride=B), :].astype(bf16)
            kv_chunk(b, j).wait()

            @pl.when(b + 1 < B)
            def _():
                kv_chunk(b + 1, j).start()

            @pl.when((b + 1 == B) & (j < _NCH - 1))
            def _():
                bwo_chunk(j).start()

            @pl.when((b + 1 == B) & (j == _NCH - 1))
            def _():
                for i in range(len(_TAIL)):
                    in_order(1, lambda _, i=i: bwo_tail(i).start())

            kk, vv = k_v.at[b % _NB], v_v.at[b % _NB]
            s = jnp.where(first, _dot_nt(q8, kk[2 * j]), _dot_nt(q8, kk[2 * j + 1]))
            m = jnp.max(s, axis=-1, keepdims=True)
            p = jnp.exp2(s - m)
            lb = jnp.sum(p, axis=-1, keepdims=True)
            pb = p.astype(bf16)
            o = jnp.where(first, _dot(pb, vv[2 * j]), _dot(pb, vv[2 * j + 1]))
            ob_s[pl.ds(pl.multiple_of(b * H + j * 2 * REP, 2 * REP), 2 * REP), :] = o / lb
            return carry2
        lax.fori_loop(0, _NCH, pair_body, 0)
        return carry

    lax.fori_loop(0, B, b_body, 0)

    def ob_heads(h0, n):
        return [ob_s[pl.ds(h0 + i, B, stride=H), :] for i in range(n)]

    def ob_body(k, acc):
        bwo_chunk(k).wait()
        return out_proj(ob_heads(k * HC, HC), bwo_v, k, acc)
    out_b = lax.fori_loop(0, _NCH - 1, ob_body, jnp.zeros((B, M), f32))
    for i, n in enumerate(_TAIL):
        lhs = jnp.concatenate(ob_heads(tail_h0[i], n), axis=-1).astype(bf16)
        bwo_tail(i).wait()
        out_b = out_b + _dot(lhs, bwo_v[pl.ds(tail_h0[i] * D, n * D), :])

    o_ref[...] = (out_a + (1.0 - gate) * out_b).astype(o_ref.dtype)


@jax.jit
def pallas_gated_mix__compressed_kv_cla__sliding_block_cached__decode_kernel(
    A_x: jax.Array,
    A_c_kv: jax.Array,
    A_w_q: jax.Array,
    A_w_uk: jax.Array,
    A_w_uv: jax.Array,
    A_w_o: jax.Array,
    B_x: jax.Array,
    B_k_cache: jax.Array,
    B_v_cache: jax.Array,
    B_wq: jax.Array,
    B_wo: jax.Array,
    gate_w: jax.Array,
):
    del B_x
    B, Sq, M = A_x.shape
    Sk, Dc = A_c_kv.shape[1], A_c_kv.shape[2]
    H, D = A_w_q.shape[1], A_w_q.shape[2]
    Hkv, Skb = B_k_cache.shape[1], B_k_cache.shape[2]
    W = min(4096, max(256, Skb // 4))
    assert Sq == 1 and B == 8 and D == 128 and Skb == Sk
    assert M == _NCH * 128 and Dc == _NCH * 128 and Hkv == 2 * _NCH and H == 4 * Hkv
    assert sum(_TAIL) == H // _NCH and len(_TAIL) >= 3 and _NB >= 2
    bf, f32 = jnp.bfloat16, jnp.float32

    kern = functools.partial(_kernel, B=B, H=H, D=D, M=M, Sk=Sk, Dc=Dc, Hkv=Hkv, W=W)
    out = pl.pallas_call(
        kern,
        out_shape=jax.ShapeDtypeStruct((B, M), A_x.dtype),
        in_specs=[pl.BlockSpec(memory_space=pl.ANY)] * 11,
        out_specs=pl.BlockSpec(memory_space=pltpu.VMEM),
        scratch_shapes=[
            pltpu.VMEM((B, M), bf),
            pltpu.VMEM((M,), bf),
            pltpu.VMEM((M * H, D), bf),
            pltpu.VMEM((Dc * H, D), bf),
            pltpu.VMEM((Dc * H, D), bf),
            pltpu.VMEM((H * D, M), bf),
            pltpu.VMEM((M, H * D), bf),
            pltpu.VMEM((H * D, M), bf),
            pltpu.VMEM((_NB, Sk, Dc), bf),
            pltpu.VMEM((_NB, Hkv, W, D), bf),
            pltpu.VMEM((_NB, Hkv, W, D), bf),
            pltpu.VMEM((H * B, D), f32),
            pltpu.VMEM((Dc // 128, H * B, 128), f32),
            pltpu.VMEM((H * B, D), f32),
            pltpu.VMEM((Dc // 128, B * H, 128), f32),
            pltpu.VMEM((B * H, D), f32),
            pltpu.VMEM((H * B, D), f32),
            pltpu.SemaphoreType.DMA((_NCH,)),
            pltpu.SemaphoreType.DMA((len(_TAIL) - 1,)),
        ],
        compiler_params=pltpu.CompilerParams(vmem_limit_bytes=80 * 2**20),
    )(
        A_x.reshape(B, M), A_c_kv,
        A_w_q.reshape(M * H, D), A_w_uk.reshape(Dc * H, D), A_w_uv.reshape(Dc * H, D),
        A_w_o.reshape(H * D, M), B_k_cache, B_v_cache, B_wq, B_wo, gate_w,
    )
    return out.reshape(B, Sq, M)
```

```python
import functools
import math

import jax
import jax.numpy as jnp
from jax import lax
import jax.experimental.pallas as pl
import jax.experimental.pallas.tpu as pltpu

_LOG2E = 1.4426950408889634
_NCH = 4
_P = 8
_NB = 2
_TAIL = (4, 2, 2)

_NT = (((1,), (1,)), ((), ()))


def _dot(a, b):
    return jnp.dot(a, b, preferred_element_type=jnp.float32)


def _dot_nt(a, b):
    return lax.dot_general(a, b, _NT, preferred_element_type=jnp.float32)


def _kernel(
    x_hbm, c_hbm, wq_hbm, wuk_hbm, wuv_hbm, wo_hbm, k_hbm, v_hbm, bwq_hbm, bwo_hbm, gw_hbm,
    o_ref,
    x_v, gw_v, wq_v, wuk_v, wuv_v, wo_v, bwq_v, bwo_v, c_v, k_v, v_v,
    qa_s, ql_s, qb_s, cl_s, ob_s, ctx_s,
    sems, tail_sems,
    *, B, H, D, M, Sk, Dc, Hkv, W,
):
    f32, bf16 = jnp.float32, jnp.bfloat16
    REP = H // Hkv
    CCH = Sk // _NCH
    CT = Dc // 128
    HP = H // 2
    HC = H // _NCH
    QC = HC * D

    class Chunk:
        def __init__(self, small, bulk):
            self.small, self.bulk = small, bulk

        def start(self, part=0, nparts=1):
            for copies, queue in ((self.small, 0), (self.bulk, 1)):
                n = len(copies)
                for copy in copies[part * n // nparts:(part + 1) * n // nparts]:
                    copy.start(priority=queue)

        def wait(self, issue=lambda part, nparts: None):
            for copy in self.small:
                copy.wait()
            for part, copy in enumerate(self.bulk):
                copy.wait()
                issue(part, len(self.bulk))

    def rows_chunk(hbm, vmem, item, k):
        n = hbm.shape[0] // _NCH
        n0 = n // 32
        n1 = n // _P - n0
        sem = sems.at[item % 2, k]

        def copy(r0, rows):
            rng = pl.ds(pl.multiple_of(k * n + r0, rows if r0 == 0 else math.gcd(n, r0)), rows)
            return pltpu.make_async_copy(hbm.at[rng], vmem.at[rng], sem)
        return Chunk([copy(i * n0, n0) for i in range(_P)],
                     [copy(_P * n0 + i * n1, n1) for i in range(_P)])

    def wq_chunk(k): return rows_chunk(wq_hbm, wq_v, 0, k)
    def wuk_chunk(k): return rows_chunk(wuk_hbm, wuk_v, 1, k)
    def c_chunk(b, k): return rows_chunk(c_hbm.at[b], c_v.at[b % _NB], 2 + b, k)
    def wuv_chunk(k): return rows_chunk(wuv_hbm, wuv_v, 2 + B, k)
    def wo_chunk(k): return rows_chunk(wo_hbm, wo_v, 3 + B, k)
    def bwo_chunk(k): return rows_chunk(bwo_hbm, bwo_v, 5 + 2 * B, k)

    def bwq_chunk(k):
        cols = pl.ds(pl.multiple_of(k * QC, QC), QC)
        n0 = M // 32
        n1 = M // _P - n0

        def copy(r0, rows):
            rng = pl.ds(r0, rows)
            return pltpu.make_async_copy(
                bwq_hbm.at[rng, cols], bwq_v.at[rng, cols], sems.at[(4 + B) % 2, k])
        return Chunk([copy(i * n0, n0) for i in range(_P)],
                     [copy(_P * n0 + i * n1, n1) for i in range(_P)])

    def kv_chunk(b, j):
        sem = sems.at[(5 + B + b) % 2, j]

        def copy(hbm, vmem, g, r0, rows):
            return pltpu.make_async_copy(hbm.at[b, g, pl.ds(Sk - W + r0, rows)],
                                         vmem.at[b % _NB, g, pl.ds(r0, rows)], sem)
        n0, n1 = W // 8, W // 2
        small = [copy(k_hbm, k_v, 2 * j, i * n0, n0) for i in range(6)]
        bulk = [copy(k_hbm, k_v, 2 * j, 6 * n0, W - 6 * n0)]
        bulk += [copy(hbm, vmem, 2 * j + g, i * n1, n1)
                 for hbm, vmem, g in ((k_hbm, k_v, 1), (v_hbm, v_v, 0), (v_hbm, v_v, 1))
                 for i in range(2)]
        return Chunk(small, bulk)

    tail_h0 = [H - HC + sum(_TAIL[:i]) for i in range(len(_TAIL))]

    def bwo_tail(i):
        sem = sems.at[(5 + 2 * B) % 2, _NCH - 1] if i == 0 else tail_sems.at[i - 1]
        n = _TAIL[i] * D // 2

        def copy(r0):
            rng = pl.ds(tail_h0[i] * D + r0, n)
            return pltpu.make_async_copy(bwo_hbm.at[rng], bwo_v.at[rng], sem)
        return Chunk([copy(0)], [copy(n)])

    def start_bwo(k, part, nparts):
        pl.when(k < _NCH - 1)(lambda: bwo_chunk(k).start(part, nparts))
        for i in range(len(_TAIL)):
            if part == i * nparts // len(_TAIL):
                pl.when(k == _NCH - 1)(bwo_tail(i).start)

    def in_order(n, start_fn):
        def body(i, carry):
            start_fn(i)
            return carry
        lax.fori_loop(0, n, body, 0)

    x_copy = pltpu.make_async_copy(x_hbm, x_v, tail_sems.at[0])
    gw_copy = pltpu.make_async_copy(gw_hbm, gw_v, tail_sems.at[1])
    x_copy.start()
    gw_copy.start()
    in_order(_NCH, lambda k: wq_chunk(k).start())

    def head_pairs(w_v, k):
        n = w_v.shape[0] // _NCH
        w = w_v[pl.ds(pl.multiple_of(k * n, n), n), :]
        u = pltpu.bitcast(w, jnp.uint32).reshape(n // H, HP, D)
        u = jnp.swapaxes(u, 0, 1)
        for p in range(HP):
            even = pltpu.bitcast(u[p] << 16, f32).astype(bf16)
            odd = pltpu.bitcast(u[p] & jnp.uint32(0xFFFF0000), f32).astype(bf16)
            yield 2 * p, even
            yield 2 * p + 1, odd

    def head_rows(h):
        return pl.ds(h * B, B)

    x_copy.wait()
    gw_copy.wait()

    qa_s[...] = jnp.zeros_like(qa_s)

    def qa_body(k, carry):
        wq_chunk(k).wait(wuk_chunk(k).start)
        xk = x_v[:, pl.ds(pl.multiple_of(k * 128, 128), 128)]
        for h, w in head_pairs(wq_v, k):
            qa_s[head_rows(h), :] += _dot(xk, w)
        return carry
    lax.fori_loop(0, _NCH, qa_body, 0)

    scale = (D ** -0.5) * _LOG2E

    def ql_body(k, carry):
        wuk_chunk(k).wait(c_chunk(0, k).start)
        for h, w in head_pairs(wuk_v, k):
            q = qa_s[head_rows(h), :].astype(bf16)
            ql_s[k, head_rows(h), :] = _dot_nt(q, w) * scale
        return carry
    lax.fori_loop(0, _NCH, ql_body, 0)

    def a_body(b, carry):
        q = jnp.concatenate(
            [ql_s[t, pl.ds(b, H, stride=B), :] for t in range(CT)], axis=-1
        ).astype(bf16)

        def chunk_body(k, mla):
            m_prev, l_prev, acc = mla
            def issue(part, nparts):
                pl.when(b + 1 < B)(lambda: c_chunk(b + 1, k).start(part, nparts))
                pl.when(b + 1 == B)(lambda: wuv_chunk(k).start(part, nparts))
            c_chunk(b, k).wait(issue)

            c = c_v[b % _NB, pl.ds(pl.multiple_of(k * CCH, CCH), CCH), :]
            s = _dot_nt(q, c)
            m_new = jnp.maximum(m_prev, jnp.max(s, axis=-1, keepdims=True))
            alpha = jnp.exp2(m_prev - m_new)
            p = jnp.exp2(s - m_new)
            l_new = alpha * l_prev + jnp.sum(p, axis=-1, keepdims=True)
            acc = alpha * acc + _dot(p.astype(bf16), c)
            return m_new, l_new, acc

        m0 = jnp.full((H, 1), -jnp.inf, f32)
        l0 = jnp.zeros((H, 1), f32)
        a0 = jnp.zeros((H, Dc), f32)
        _, l, acc = lax.fori_loop(0, _NCH, chunk_body, (m0, l0, a0))
        cl = acc / l
        for t in range(CT):
            cl_s[t, pl.ds(pl.multiple_of(b * H, H), H), :] = cl[:, t * 128:(t + 1) * 128]
        return carry

    lax.fori_loop(0, B, a_body, 0)

    ctx_s[...] = jnp.zeros_like(ctx_s)

    def ctx_body(k, carry):
        wuv_chunk(k).wait(wo_chunk(k).start)
        for h, w in head_pairs(wuv_v, k):
            lhs = cl_s[k, pl.ds(h, B, stride=H), :].astype(bf16)
            ctx_s[head_rows(h), :] += _dot(lhs, w)
        return carry
    lax.fori_loop(0, _NCH, ctx_body, 0)

    def out_proj(lhs_heads, w_v, k, acc):
        lhs = jnp.concatenate(lhs_heads, axis=-1).astype(bf16)
        n = w_v.shape[0] // _NCH
        return acc + _dot(lhs, w_v[pl.ds(pl.multiple_of(k * n, n), n), :])

    def oa_body(k, acc):
        wo_chunk(k).wait(bwq_chunk(k).start)
        lhs = [ctx_s[pl.ds(pl.multiple_of((k * HC + i) * B, B), B), :] for i in range(HC)]
        return out_proj(lhs, wo_v, k, acc)
    out_a = lax.fori_loop(0, _NCH, oa_body, jnp.zeros((B, M), f32))

    gate_logit = jnp.sum(x_v[...].astype(f32) * gw_v[...].astype(f32).reshape(1, M),
                         axis=-1, keepdims=True)
    gate = jax.nn.sigmoid(gate_logit)
    out_a = gate * out_a

    def qb_body(k, carry):
        bwq_chunk(k).wait(kv_chunk(0, k).start)
        q = _dot(x_v[...], bwq_v[:, pl.ds(pl.multiple_of(k * QC, QC), QC)]) * scale
        for i in range(HC):
            qb_s[pl.ds(pl.multiple_of((k * HC + i) * B, B), B), :] = q[:, i * D:(i + 1) * D]
        return carry
    lax.fori_loop(0, _NCH, qb_body, 0)

    first = lax.broadcasted_iota(jnp.int32, (2 * REP, 1), 0) < REP

    def b_body(b, carry):
        def pair_body(j, carry2):
            q8 = qb_s[pl.ds(j * 2 * REP * B + b, 2 * REP, stride=B), :].astype(bf16)
            def issue(part, nparts):
                pl.when(b + 1 < B)(lambda: kv_chunk(b + 1, j).start(part, nparts))
                pl.when(b + 1 == B)(lambda: start_bwo(j, part, nparts))
            kv_chunk(b, j).wait(issue)

            kk, vv = k_v.at[b % _NB], v_v.at[b % _NB]
            s = jnp.where(first, _dot_nt(q8, kk[2 * j]), _dot_nt(q8, kk[2 * j + 1]))
            m = jnp.max(s, axis=-1, keepdims=True)
            p = jnp.exp2(s - m)
            lb = jnp.sum(p, axis=-1, keepdims=True)
            pb = p.astype(bf16)
            o = jnp.where(first, _dot(pb, vv[2 * j]), _dot(pb, vv[2 * j + 1]))
            ob_s[pl.ds(pl.multiple_of(b * H + j * 2 * REP, 2 * REP), 2 * REP), :] = o / lb
            return carry2
        lax.fori_loop(0, _NCH, pair_body, 0)
        return carry

    lax.fori_loop(0, B, b_body, 0)

    def ob_heads(h0, n):
        return [ob_s[pl.ds(h0 + i, B, stride=H), :] for i in range(n)]

    def ob_body(k, acc):
        bwo_chunk(k).wait()
        return out_proj(ob_heads(k * HC, HC), bwo_v, k, acc)
    out_b = lax.fori_loop(0, _NCH - 1, ob_body, jnp.zeros((B, M), f32))
    for i, n in enumerate(_TAIL):
        lhs = jnp.concatenate(ob_heads(tail_h0[i], n), axis=-1).astype(bf16)
        bwo_tail(i).wait()
        out_b = out_b + _dot(lhs, bwo_v[pl.ds(tail_h0[i] * D, n * D), :])

    o_ref[...] = (out_a + (1.0 - gate) * out_b).astype(o_ref.dtype)


@jax.jit
def pallas_gated_mix__compressed_kv_cla__sliding_block_cached__decode_kernel(
    A_x: jax.Array,
    A_c_kv: jax.Array,
    A_w_q: jax.Array,
    A_w_uk: jax.Array,
    A_w_uv: jax.Array,
    A_w_o: jax.Array,
    B_x: jax.Array,
    B_k_cache: jax.Array,
    B_v_cache: jax.Array,
    B_wq: jax.Array,
    B_wo: jax.Array,
    gate_w: jax.Array,
):
    del B_x
    B, Sq, M = A_x.shape
    Sk, Dc = A_c_kv.shape[1], A_c_kv.shape[2]
    H, D = A_w_q.shape[1], A_w_q.shape[2]
    Hkv, Skb = B_k_cache.shape[1], B_k_cache.shape[2]
    W = min(4096, max(256, Skb // 4))
    assert Sq == 1 and B == 8 and D == 128 and Skb == Sk
    assert M == _NCH * 128 and Dc == _NCH * 128 and Hkv == 2 * _NCH and H == 4 * Hkv
    assert sum(_TAIL) == H // _NCH and len(_TAIL) >= 3 and _NB >= 2
    bf, f32 = jnp.bfloat16, jnp.float32

    kern = functools.partial(_kernel, B=B, H=H, D=D, M=M, Sk=Sk, Dc=Dc, Hkv=Hkv, W=W)
    out = pl.pallas_call(
        kern,
        out_shape=jax.ShapeDtypeStruct((B, M), A_x.dtype),
        in_specs=[pl.BlockSpec(memory_space=pl.ANY)] * 11,
        out_specs=pl.BlockSpec(memory_space=pltpu.VMEM),
        scratch_shapes=[
            pltpu.VMEM((B, M), bf),
            pltpu.VMEM((M,), bf),
            pltpu.VMEM((M * H, D), bf),
            pltpu.VMEM((Dc * H, D), bf),
            pltpu.VMEM((Dc * H, D), bf),
            pltpu.VMEM((H * D, M), bf),
            pltpu.VMEM((M, H * D), bf),
            pltpu.VMEM((H * D, M), bf),
            pltpu.VMEM((_NB, Sk, Dc), bf),
            pltpu.VMEM((_NB, Hkv, W, D), bf),
            pltpu.VMEM((_NB, Hkv, W, D), bf),
            pltpu.VMEM((H * B, D), f32),
            pltpu.VMEM((Dc // 128, H * B, 128), f32),
            pltpu.VMEM((H * B, D), f32),
            pltpu.VMEM((Dc // 128, B * H, 128), f32),
            pltpu.VMEM((B * H, D), f32),
            pltpu.VMEM((H * B, D), f32),
            pltpu.SemaphoreType.DMA((2, _NCH)),
            pltpu.SemaphoreType.DMA((len(_TAIL) - 1,)),
        ],
        compiler_params=pltpu.CompilerParams(vmem_limit_bytes=80 * 2**20),
    )(
        A_x.reshape(B, M), A_c_kv,
        A_w_q.reshape(M * H, D), A_w_uk.reshape(Dc * H, D), A_w_uv.reshape(Dc * H, D),
        A_w_o.reshape(H * D, M), B_k_cache, B_v_cache, B_wq, B_wo, gate_w,
    )
    return out.reshape(B, Sq, M)
```

```python
import functools
import math

import jax
import jax.numpy as jnp
from jax import lax
import jax.experimental.pallas as pl
import jax.experimental.pallas.tpu as pltpu

_LOG2E = 1.4426950408889634
_NCH = 4
_P = 8
_NB = 2
_TAIL = (4, 2, 2)

_NT = (((1,), (1,)), ((), ()))


def _dot(a, b):
    return jnp.dot(a, b, preferred_element_type=jnp.float32)


def _dot_nt(a, b):
    return lax.dot_general(a, b, _NT, preferred_element_type=jnp.float32)


def _kernel(
    x_hbm, c_hbm, wq_hbm, wuk_hbm, wuv_hbm, wo_hbm, k_hbm, v_hbm, bwq_hbm, bwo_hbm, gw_hbm,
    o_ref,
    x_v, gw_v, wq_v, wuk_v, wuv_v, wo_v, bwq_v, bwo_v, c_v, k_v, v_v,
    qa_s, ql_s, qb_s, cl_s, ob_s, ctx_s,
    sems, tail_sems,
    *, B, H, D, M, Sk, Dc, Hkv, W,
):
    f32, bf16 = jnp.float32, jnp.bfloat16
    REP = H // Hkv
    CCH = Sk // _NCH
    CT = Dc // 128
    HP = H // 2
    HC = H // _NCH
    QC = HC * D

    class Chunk:
        def __init__(self, copy, small, bulk):
            self.copy = copy
            self.small, self.bulk = small, bulk

        def start(self, part=0, nparts=1):
            for pieces, queue in ((self.small, 0), (self.bulk, 1)):
                n = len(pieces)
                for piece in pieces[part * n // nparts:(part + 1) * n // nparts]:
                    self.copy(*piece).start(priority=queue)

        def wait(self, issue=lambda part, nparts: None):
            for piece in self.small:
                self.copy(*piece).wait()
            for part, piece in enumerate(self.bulk):
                self.copy(*piece).wait()
                issue(part, len(self.bulk))

    def row_pieces(n):
        n0 = n // 32
        n1 = n // _P - n0
        return ([(i * n0, n0) for i in range(_P)],
                [(_P * n0 + i * n1, n1) for i in range(_P)])

    def rows_chunk(hbm, vmem, item, k):
        n = hbm.shape[0] // _NCH

        def copy(r0, rows):
            rng = pl.ds(pl.multiple_of(k * n + r0, math.gcd(n, r0)), rows)
            return pltpu.make_async_copy(hbm.at[rng], vmem.at[rng], sems.at[item % 2, k])
        return Chunk(copy, *row_pieces(n))

    def wq_chunk(k): return rows_chunk(wq_hbm, wq_v, 0, k)
    def wuk_chunk(k): return rows_chunk(wuk_hbm, wuk_v, 1, k)
    def c_chunk(b, k): return rows_chunk(c_hbm.at[b], c_v.at[b % _NB], 2 + b, k)
    def wuv_chunk(k): return rows_chunk(wuv_hbm, wuv_v, 2 + B, k)
    def wo_chunk(k): return rows_chunk(wo_hbm, wo_v, 3 + B, k)
    def bwo_chunk(k): return rows_chunk(bwo_hbm, bwo_v, 5 + 2 * B, k)

    def bwq_chunk(k):
        cols = pl.ds(pl.multiple_of(k * QC, QC), QC)

        def copy(r0, rows):
            rng = pl.ds(r0, rows)
            return pltpu.make_async_copy(
                bwq_hbm.at[rng, cols], bwq_v.at[rng, cols], sems.at[(4 + B) % 2, k])
        return Chunk(copy, *row_pieces(M))

    def kv_chunk(b, j):
        def copy(hbm, vmem, g, r0, rows):
            return pltpu.make_async_copy(
                hbm.at[b, 2 * j + g, pl.ds(Sk - W + r0, rows)],
                vmem.at[b % _NB, 2 * j + g, pl.ds(r0, rows)], sems.at[(5 + B + b) % 2, j])
        n0, n1 = W // 8, W // 2
        small = [(k_hbm, k_v, 0, i * n0, n0) for i in range(6)]
        bulk = [(k_hbm, k_v, 0, 6 * n0, W - 6 * n0)]
        bulk += [(hbm, vmem, g, i * n1, n1)
                 for hbm, vmem, g in ((k_hbm, k_v, 1), (v_hbm, v_v, 0), (v_hbm, v_v, 1))
                 for i in range(2)]
        return Chunk(copy, small, bulk)

    tail_h0 = [H - HC + sum(_TAIL[:i]) for i in range(len(_TAIL))]

    def bwo_tail(i):
        n = _TAIL[i] * D // 2

        def copy(r0):
            sem = sems.at[(5 + 2 * B) % 2, _NCH - 1] if i == 0 else tail_sems.at[i - 1]
            rng = pl.ds(tail_h0[i] * D + r0, n)
            return pltpu.make_async_copy(bwo_hbm.at[rng], bwo_v.at[rng], sem)
        return Chunk(copy, [(0,)], [(n,)])

    def start_bwo(k, part, nparts):
        pl.when(k < _NCH - 1)(lambda: bwo_chunk(k).start(part, nparts))
        for i in range(len(_TAIL)):
            if part == i * nparts // len(_TAIL):
                pl.when(k == _NCH - 1)(lambda i=i: bwo_tail(i).start())

    def in_order(n, start_fn):
        def body(i, carry):
            start_fn(i)
            return carry
        lax.fori_loop(0, n, body, 0)

    x_copy = pltpu.make_async_copy(x_hbm, x_v, tail_sems.at[0])
    gw_copy = pltpu.make_async_copy(gw_hbm, gw_v, tail_sems.at[1])
    x_copy.start()
    gw_copy.start()
    in_order(_NCH, lambda k: wq_chunk(k).start())

    def head_pairs(w_v, k):
        n = w_v.shape[0] // _NCH
        w = w_v[pl.ds(pl.multiple_of(k * n, n), n), :]
        u = pltpu.bitcast(w, jnp.uint32).reshape(n // H, HP, D)
        u = jnp.swapaxes(u, 0, 1)
        for p in range(HP):
            even = pltpu.bitcast(u[p] << 16, f32).astype(bf16)
            odd = pltpu.bitcast(u[p] & jnp.uint32(0xFFFF0000), f32).astype(bf16)
            yield 2 * p, even
            yield 2 * p + 1, odd

    def head_rows(h):
        return pl.ds(h * B, B)

    x_copy.wait()
    gw_copy.wait()

    qa_s[...] = jnp.zeros_like(qa_s)

    def qa_body(k, carry):
        wq_chunk(k).wait(wuk_chunk(k).start)
        xk = x_v[:, pl.ds(pl.multiple_of(k * 128, 128), 128)]
        for h, w in head_pairs(wq_v, k):
            qa_s[head_rows(h), :] += _dot(xk, w)
        return carry
    lax.fori_loop(0, _NCH, qa_body, 0)

    scale = (D ** -0.5) * _LOG2E

    def ql_body(k, carry):
        wuk_chunk(k).wait(c_chunk(0, k).start)
        for h, w in head_pairs(wuk_v, k):
            q = qa_s[head_rows(h), :].astype(bf16)
            ql_s[k, head_rows(h), :] = _dot_nt(q, w) * scale
        return carry
    lax.fori_loop(0, _NCH, ql_body, 0)

    def a_body(b, carry):
        q = jnp.concatenate(
            [ql_s[t, pl.ds(b, H, stride=B), :] for t in range(CT)], axis=-1
        ).astype(bf16)

        def chunk_body(k, mla):
            m_prev, l_prev, acc = mla
            def issue(part, nparts):
                pl.when(b + 1 < B)(lambda: c_chunk(b + 1, k).start(part, nparts))
                pl.when(b + 1 == B)(lambda: wuv_chunk(k).start(part, nparts))
            c_chunk(b, k).wait(issue)

            c = c_v[b % _NB, pl.ds(pl.multiple_of(k * CCH, CCH), CCH), :]
            s = _dot_nt(q, c)
            m_new = jnp.maximum(m_prev, jnp.max(s, axis=-1, keepdims=True))
            alpha = jnp.exp2(m_prev - m_new)
            p = jnp.exp2(s - m_new)
            l_new = alpha * l_prev + jnp.sum(p, axis=-1, keepdims=True)
            acc = alpha * acc + _dot(p.astype(bf16), c)
            return m_new, l_new, acc

        m0 = jnp.full((H, 1), -jnp.inf, f32)
        l0 = jnp.zeros((H, 1), f32)
        a0 = jnp.zeros((H, Dc), f32)
        _, l, acc = lax.fori_loop(0, _NCH, chunk_body, (m0, l0, a0))
        cl = acc / l
        for t in range(CT):
            cl_s[t, pl.ds(pl.multiple_of(b * H, H), H), :] = cl[:, t * 128:(t + 1) * 128]
        return carry

    lax.fori_loop(0, B, a_body, 0)

    ctx_s[...] = jnp.zeros_like(ctx_s)

    def ctx_body(k, carry):
        wuv_chunk(k).wait(wo_chunk(k).start)
        for h, w in head_pairs(wuv_v, k):
            lhs = cl_s[k, pl.ds(h, B, stride=H), :].astype(bf16)
            ctx_s[head_rows(h), :] += _dot(lhs, w)
        return carry
    lax.fori_loop(0, _NCH, ctx_body, 0)

    def out_proj(lhs_heads, w_v, k, acc):
        lhs = jnp.concatenate(lhs_heads, axis=-1).astype(bf16)
        n = w_v.shape[0] // _NCH
        return acc + _dot(lhs, w_v[pl.ds(pl.multiple_of(k * n, n), n), :])

    def oa_body(k, acc):
        wo_chunk(k).wait(bwq_chunk(k).start)
        lhs = [ctx_s[pl.ds(pl.multiple_of((k * HC + i) * B, B), B), :] for i in range(HC)]
        return out_proj(lhs, wo_v, k, acc)
    out_a = lax.fori_loop(0, _NCH, oa_body, jnp.zeros((B, M), f32))

    gate_logit = jnp.sum(x_v[...].astype(f32) * gw_v[...].astype(f32).reshape(1, M),
                         axis=-1, keepdims=True)
    gate = jax.nn.sigmoid(gate_logit)
    out_a = gate * out_a

    def qb_body(k, carry):
        bwq_chunk(k).wait(kv_chunk(0, k).start)
        q = _dot(x_v[...], bwq_v[:, pl.ds(pl.multiple_of(k * QC, QC), QC)]) * scale
        for i in range(HC):
            qb_s[pl.ds(pl.multiple_of((k * HC + i) * B, B), B), :] = q[:, i * D:(i + 1) * D]
        return carry
    lax.fori_loop(0, _NCH, qb_body, 0)

    first = lax.broadcasted_iota(jnp.int32, (2 * REP, 1), 0) < REP

    def b_body(b, carry):
        def pair_body(j, carry2):
            q8 = qb_s[pl.ds(j * 2 * REP * B + b, 2 * REP, stride=B), :].astype(bf16)
            def issue(part, nparts):
                pl.when(b + 1 < B)(lambda: kv_chunk(b + 1, j).start(part, nparts))
                pl.when(b + 1 == B)(lambda: start_bwo(j, part, nparts))
            kv_chunk(b, j).wait(issue)

            kk, vv = k_v.at[b % _NB], v_v.at[b % _NB]
            s = jnp.where(first, _dot_nt(q8, kk[2 * j]), _dot_nt(q8, kk[2 * j + 1]))
            m = jnp.max(s, axis=-1, keepdims=True)
            p = jnp.exp2(s - m)
            lb = jnp.sum(p, axis=-1, keepdims=True)
            pb = p.astype(bf16)
            o = jnp.where(first, _dot(pb, vv[2 * j]), _dot(pb, vv[2 * j + 1]))
            ob_s[pl.ds(pl.multiple_of(b * H + j * 2 * REP, 2 * REP), 2 * REP), :] = o / lb
            return carry2
        lax.fori_loop(0, _NCH, pair_body, 0)
        return carry

    lax.fori_loop(0, B, b_body, 0)

    def ob_heads(h0, n):
        return [ob_s[pl.ds(h0 + i, B, stride=H), :] for i in range(n)]

    def ob_body(k, acc):
        bwo_chunk(k).wait()
        return out_proj(ob_heads(k * HC, HC), bwo_v, k, acc)
    out_b = lax.fori_loop(0, _NCH - 1, ob_body, jnp.zeros((B, M), f32))
    for i, n in enumerate(_TAIL):
        lhs = jnp.concatenate(ob_heads(tail_h0[i], n), axis=-1).astype(bf16)
        bwo_tail(i).wait()
        out_b = out_b + _dot(lhs, bwo_v[pl.ds(tail_h0[i] * D, n * D), :])

    o_ref[...] = (out_a + (1.0 - gate) * out_b).astype(o_ref.dtype)


@jax.jit
def pallas_gated_mix__compressed_kv_cla__sliding_block_cached__decode_kernel(
    A_x: jax.Array,
    A_c_kv: jax.Array,
    A_w_q: jax.Array,
    A_w_uk: jax.Array,
    A_w_uv: jax.Array,
    A_w_o: jax.Array,
    B_x: jax.Array,
    B_k_cache: jax.Array,
    B_v_cache: jax.Array,
    B_wq: jax.Array,
    B_wo: jax.Array,
    gate_w: jax.Array,
):
    del B_x
    B, Sq, M = A_x.shape
    Sk, Dc = A_c_kv.shape[1], A_c_kv.shape[2]
    H, D = A_w_q.shape[1], A_w_q.shape[2]
    Hkv, Skb = B_k_cache.shape[1], B_k_cache.shape[2]
    W = min(4096, max(256, Skb // 4))
    assert Sq == 1 and B == 8 and D == 128 and Skb == Sk
    assert M == _NCH * 128 and Dc == _NCH * 128 and Hkv == 2 * _NCH and H == 4 * Hkv
    assert sum(_TAIL) == H // _NCH and len(_TAIL) >= 3 and _NB >= 2
    bf, f32 = jnp.bfloat16, jnp.float32

    kern = functools.partial(_kernel, B=B, H=H, D=D, M=M, Sk=Sk, Dc=Dc, Hkv=Hkv, W=W)
    out = pl.pallas_call(
        kern,
        out_shape=jax.ShapeDtypeStruct((B, M), A_x.dtype),
        in_specs=[pl.BlockSpec(memory_space=pl.ANY)] * 11,
        out_specs=pl.BlockSpec(memory_space=pltpu.VMEM),
        scratch_shapes=[
            pltpu.VMEM((B, M), bf),
            pltpu.VMEM((M,), bf),
            pltpu.VMEM((M * H, D), bf),
            pltpu.VMEM((Dc * H, D), bf),
            pltpu.VMEM((Dc * H, D), bf),
            pltpu.VMEM((H * D, M), bf),
            pltpu.VMEM((M, H * D), bf),
            pltpu.VMEM((H * D, M), bf),
            pltpu.VMEM((_NB, Sk, Dc), bf),
            pltpu.VMEM((_NB, Hkv, W, D), bf),
            pltpu.VMEM((_NB, Hkv, W, D), bf),
            pltpu.VMEM((H * B, D), f32),
            pltpu.VMEM((Dc // 128, H * B, 128), f32),
            pltpu.VMEM((H * B, D), f32),
            pltpu.VMEM((Dc // 128, B * H, 128), f32),
            pltpu.VMEM((B * H, D), f32),
            pltpu.VMEM((H * B, D), f32),
            pltpu.SemaphoreType.DMA((2, _NCH)),
            pltpu.SemaphoreType.DMA((len(_TAIL) - 1,)),
        ],
        compiler_params=pltpu.CompilerParams(vmem_limit_bytes=80 * 2**20),
    )(
        A_x.reshape(B, M), A_c_kv,
        A_w_q.reshape(M * H, D), A_w_uk.reshape(Dc * H, D), A_w_uv.reshape(Dc * H, D),
        A_w_o.reshape(H * D, M), B_k_cache, B_v_cache, B_wq, B_wo, gate_w,
    )
    return out.reshape(B, Sq, M)
```

```python
import functools
import math

import jax
import jax.numpy as jnp
from jax import lax
import jax.experimental.pallas as pl
import jax.experimental.pallas.tpu as pltpu

_LOG2E = 1.4426950408889634
_NCH = 4
_NPC = 32
_NPC0 = 16
_NB = 2
_TAIL = (4, 2, 2)

_NT = (((1,), (1,)), ((), ()))


def _dot(a, b):
    return jnp.dot(a, b, preferred_element_type=jnp.float32)


def _dot_nt(a, b):
    return lax.dot_general(a, b, _NT, preferred_element_type=jnp.float32)


def _kernel(
    x_hbm, c_hbm, wq_hbm, wuk_hbm, wuv_hbm, wo_hbm, k_hbm, v_hbm, bwq_hbm, bwo_hbm, gw_hbm,
    o_ref,
    x_v, gw_v, wq_v, wuk_v, wuv_v, wo_v, bwq_v, bwo_v, c_v, k_v, v_v,
    qa_s, ql_s, qb_s, cl_s, ob_s, ctx_s,
    sems, tail_sems,
    *, B, H, D, M, Sk, Dc, Hkv, W,
):
    f32, bf16 = jnp.float32, jnp.bfloat16
    REP = H // Hkv
    CCH = Sk // _NCH
    CT = Dc // 128
    HP = H // 2
    HC = H // _NCH
    QC = HC * D

    class Chunk:
        def __init__(self, copy, small, bulk):
            self.copy = copy
            self.small, self.bulk = small, bulk

        def start(self, part=0, nparts=1):
            for pieces, queue in ((self.small, 0), (self.bulk, 1)):
                n = len(pieces)
                for piece in pieces[part * n // nparts:(part + 1) * n // nparts]:
                    self.copy(*piece).start(priority=queue)

        def wait(self, issue=lambda part, nparts: None):
            for piece in self.small:
                self.copy(*piece).wait()
            for part, piece in enumerate(self.bulk):
                self.copy(*piece).wait()
                issue(part, len(self.bulk))

    def split(pieces):
        return pieces[:_NPC0], pieces[_NPC0:]

    def row_pieces(n):
        return split([(i * (n // _NPC), n // _NPC) for i in range(_NPC)])

    def rows_chunk(hbm, vmem, item, k):
        n = hbm.shape[0] // _NCH

        def copy(r0, rows):
            rng = pl.ds(pl.multiple_of(k * n + r0, math.gcd(n, r0)), rows)
            return pltpu.make_async_copy(hbm.at[rng], vmem.at[rng], sems.at[item % 2, k])
        return Chunk(copy, *row_pieces(n))

    def wq_chunk(k): return rows_chunk(wq_hbm, wq_v, 0, k)
    def wuk_chunk(k): return rows_chunk(wuk_hbm, wuk_v, 1, k)
    def c_chunk(b, k): return rows_chunk(c_hbm.at[b], c_v.at[b % _NB], 2 + b, k)
    def wuv_chunk(k): return rows_chunk(wuv_hbm, wuv_v, 2 + B, k)
    def wo_chunk(k): return rows_chunk(wo_hbm, wo_v, 3 + B, k)
    def bwo_chunk(k): return rows_chunk(bwo_hbm, bwo_v, 5 + 2 * B, k)

    def bwq_chunk(k):
        cols = pl.ds(pl.multiple_of(k * QC, QC), QC)

        def copy(r0, rows):
            rng = pl.ds(r0, rows)
            return pltpu.make_async_copy(
                bwq_hbm.at[rng, cols], bwq_v.at[rng, cols], sems.at[(4 + B) % 2, k])
        return Chunk(copy, *row_pieces(M))

    def kv_chunk(b, j):
        def copy(hbm, vmem, g, r0, rows):
            return pltpu.make_async_copy(
                hbm.at[b, 2 * j + g, pl.ds(Sk - W + r0, rows)],
                vmem.at[b % _NB, 2 * j + g, pl.ds(r0, rows)], sems.at[(5 + B + b) % 2, j])
        return Chunk(copy, *split([
            (hbm, vmem, g, i * (4 * W // _NPC), 4 * W // _NPC)
            for hbm, vmem in ((k_hbm, k_v), (v_hbm, v_v)) for g in range(2)
            for i in range(_NPC // 4)]))

    tail_h0 = [H - HC + sum(_TAIL[:i]) for i in range(len(_TAIL))]

    def bwo_tail(i):
        n = _TAIL[i] * D // 2

        def copy(r0):
            sem = sems.at[(5 + 2 * B) % 2, _NCH - 1] if i == 0 else tail_sems.at[i - 1]
            rng = pl.ds(tail_h0[i] * D + r0, n)
            return pltpu.make_async_copy(bwo_hbm.at[rng], bwo_v.at[rng], sem)
        return Chunk(copy, [(0,)], [(n,)])

    def start_bwo(k, part, nparts):
        pl.when(k < _NCH - 1)(lambda: bwo_chunk(k).start(part, nparts))
        for i in range(len(_TAIL)):
            if part == i * nparts // len(_TAIL):
                pl.when(k == _NCH - 1)(lambda i=i: bwo_tail(i).start())

    def in_order(n, start_fn):
        def body(i, carry):
            start_fn(i)
            return carry
        lax.fori_loop(0, n, body, 0)

    x_copy = pltpu.make_async_copy(x_hbm, x_v, tail_sems.at[0])
    gw_copy = pltpu.make_async_copy(gw_hbm, gw_v, tail_sems.at[1])
    x_copy.start()
    gw_copy.start()
    in_order(_NCH, lambda k: wq_chunk(k).start())

    def head_pairs(w_v, k):
        n = w_v.shape[0] // _NCH
        w = w_v[pl.ds(pl.multiple_of(k * n, n), n), :]
        u = pltpu.bitcast(w, jnp.uint32).reshape(n // H, HP, D)
        u = jnp.swapaxes(u, 0, 1)
        for p in range(HP):
            even = pltpu.bitcast(u[p] << 16, f32).astype(bf16)
            odd = pltpu.bitcast(u[p] & jnp.uint32(0xFFFF0000), f32).astype(bf16)
            yield 2 * p, even
            yield 2 * p + 1, odd

    def head_rows(h):
        return pl.ds(h * B, B)

    x_copy.wait()
    gw_copy.wait()

    qa_s[...] = jnp.zeros_like(qa_s)

    def qa_body(k, carry):
        wq_chunk(k).wait(wuk_chunk(k).start)
        xk = x_v[:, pl.ds(pl.multiple_of(k * 128, 128), 128)]
        for h, w in head_pairs(wq_v, k):
            qa_s[head_rows(h), :] += _dot(xk, w)
        return carry
    lax.fori_loop(0, _NCH, qa_body, 0)

    scale = (D ** -0.5) * _LOG2E

    def ql_body(k, carry):
        wuk_chunk(k).wait(c_chunk(0, k).start)
        for h, w in head_pairs(wuk_v, k):
            q = qa_s[head_rows(h), :].astype(bf16)
            ql_s[k, head_rows(h), :] = _dot_nt(q, w) * scale
        return carry
    lax.fori_loop(0, _NCH, ql_body, 0)

    def a_body(b, carry):
        q = jnp.concatenate(
            [ql_s[t, pl.ds(b, H, stride=B), :] for t in range(CT)], axis=-1
        ).astype(bf16)

        def chunk_body(k, mla):
            m_prev, l_prev, acc = mla
            def issue(part, nparts):
                pl.when(b + 1 < B)(lambda: c_chunk(b + 1, k).start(part, nparts))
                pl.when(b + 1 == B)(lambda: wuv_chunk(k).start(part, nparts))
            c_chunk(b, k).wait(issue)

            c = c_v[b % _NB, pl.ds(pl.multiple_of(k * CCH, CCH), CCH), :]
            s = _dot_nt(q, c)
            m_new = jnp.maximum(m_prev, jnp.max(s, axis=-1, keepdims=True))
            alpha = jnp.exp2(m_prev - m_new)
            p = jnp.exp2(s - m_new)
            l_new = alpha * l_prev + jnp.sum(p, axis=-1, keepdims=True)
            acc = alpha * acc + _dot(p.astype(bf16), c)
            return m_new, l_new, acc

        m0 = jnp.full((H, 1), -jnp.inf, f32)
        l0 = jnp.zeros((H, 1), f32)
        a0 = jnp.zeros((H, Dc), f32)
        _, l, acc = lax.fori_loop(0, _NCH, chunk_body, (m0, l0, a0))
        cl = acc / l
        for t in range(CT):
            cl_s[t, pl.ds(pl.multiple_of(b * H, H), H), :] = cl[:, t * 128:(t + 1) * 128]
        return carry

    lax.fori_loop(0, B, a_body, 0)

    ctx_s[...] = jnp.zeros_like(ctx_s)

    def ctx_body(k, carry):
        wuv_chunk(k).wait(wo_chunk(k).start)
        for h, w in head_pairs(wuv_v, k):
            lhs = cl_s[k, pl.ds(h, B, stride=H), :].astype(bf16)
            ctx_s[head_rows(h), :] += _dot(lhs, w)
        return carry
    lax.fori_loop(0, _NCH, ctx_body, 0)

    def out_proj(lhs_heads, w_v, k, acc):
        lhs = jnp.concatenate(lhs_heads, axis=-1).astype(bf16)
        n = w_v.shape[0] // _NCH
        return acc + _dot(lhs, w_v[pl.ds(pl.multiple_of(k * n, n), n), :])

    def oa_body(k, acc):
        wo_chunk(k).wait(bwq_chunk(k).start)
        lhs = [ctx_s[pl.ds(pl.multiple_of((k * HC + i) * B, B), B), :] for i in range(HC)]
        return out_proj(lhs, wo_v, k, acc)
    out_a = lax.fori_loop(0, _NCH, oa_body, jnp.zeros((B, M), f32))

    gate_logit = jnp.sum(x_v[...].astype(f32) * gw_v[...].astype(f32).reshape(1, M),
                         axis=-1, keepdims=True)
    gate = jax.nn.sigmoid(gate_logit)
    out_a = gate * out_a

    def qb_body(k, carry):
        bwq_chunk(k).wait(kv_chunk(0, k).start)
        q = _dot(x_v[...], bwq_v[:, pl.ds(pl.multiple_of(k * QC, QC), QC)]) * scale
        for i in range(HC):
            qb_s[pl.ds(pl.multiple_of((k * HC + i) * B, B), B), :] = q[:, i * D:(i + 1) * D]
        return carry
    lax.fori_loop(0, _NCH, qb_body, 0)

    first = lax.broadcasted_iota(jnp.int32, (2 * REP, 1), 0) < REP

    def b_body(b, carry):
        def pair_body(j, carry2):
            q8 = qb_s[pl.ds(j * 2 * REP * B + b, 2 * REP, stride=B), :].astype(bf16)
            def issue(part, nparts):
                pl.when(b + 1 < B)(lambda: kv_chunk(b + 1, j).start(part, nparts))
                pl.when(b + 1 == B)(lambda: start_bwo(j, part, nparts))
            kv_chunk(b, j).wait(issue)

            kk, vv = k_v.at[b % _NB], v_v.at[b % _NB]
            s = jnp.where(first, _dot_nt(q8, kk[2 * j]), _dot_nt(q8, kk[2 * j + 1]))
            m = jnp.max(s, axis=-1, keepdims=True)
            p = jnp.exp2(s - m)
            lb = jnp.sum(p, axis=-1, keepdims=True)
            pb = p.astype(bf16)
            o = jnp.where(first, _dot(pb, vv[2 * j]), _dot(pb, vv[2 * j + 1]))
            ob_s[pl.ds(pl.multiple_of(b * H + j * 2 * REP, 2 * REP), 2 * REP), :] = o / lb
            return carry2
        lax.fori_loop(0, _NCH, pair_body, 0)
        return carry

    lax.fori_loop(0, B, b_body, 0)

    def ob_heads(h0, n):
        return [ob_s[pl.ds(h0 + i, B, stride=H), :] for i in range(n)]

    def ob_body(k, acc):
        bwo_chunk(k).wait()
        return out_proj(ob_heads(k * HC, HC), bwo_v, k, acc)
    out_b = lax.fori_loop(0, _NCH - 1, ob_body, jnp.zeros((B, M), f32))
    for i, n in enumerate(_TAIL):
        lhs = jnp.concatenate(ob_heads(tail_h0[i], n), axis=-1).astype(bf16)
        bwo_tail(i).wait()
        out_b = out_b + _dot(lhs, bwo_v[pl.ds(tail_h0[i] * D, n * D), :])

    o_ref[...] = (out_a + (1.0 - gate) * out_b).astype(o_ref.dtype)


@jax.jit
def pallas_gated_mix__compressed_kv_cla__sliding_block_cached__decode_kernel(
    A_x: jax.Array,
    A_c_kv: jax.Array,
    A_w_q: jax.Array,
    A_w_uk: jax.Array,
    A_w_uv: jax.Array,
    A_w_o: jax.Array,
    B_x: jax.Array,
    B_k_cache: jax.Array,
    B_v_cache: jax.Array,
    B_wq: jax.Array,
    B_wo: jax.Array,
    gate_w: jax.Array,
):
    del B_x
    B, Sq, M = A_x.shape
    Sk, Dc = A_c_kv.shape[1], A_c_kv.shape[2]
    H, D = A_w_q.shape[1], A_w_q.shape[2]
    Hkv, Skb = B_k_cache.shape[1], B_k_cache.shape[2]
    W = min(4096, max(256, Skb // 4))
    assert Sq == 1 and B == 8 and D == 128 and Skb == Sk
    assert M == _NCH * 128 and Dc == _NCH * 128 and Hkv == 2 * _NCH and H == 4 * Hkv
    assert sum(_TAIL) == H // _NCH and len(_TAIL) >= 3 and _NB >= 2
    bf, f32 = jnp.bfloat16, jnp.float32

    kern = functools.partial(_kernel, B=B, H=H, D=D, M=M, Sk=Sk, Dc=Dc, Hkv=Hkv, W=W)
    out = pl.pallas_call(
        kern,
        out_shape=jax.ShapeDtypeStruct((B, M), A_x.dtype),
        in_specs=[pl.BlockSpec(memory_space=pl.ANY)] * 11,
        out_specs=pl.BlockSpec(memory_space=pltpu.VMEM),
        scratch_shapes=[
            pltpu.VMEM((B, M), bf),
            pltpu.VMEM((M,), bf),
            pltpu.VMEM((M * H, D), bf),
            pltpu.VMEM((Dc * H, D), bf),
            pltpu.VMEM((Dc * H, D), bf),
            pltpu.VMEM((H * D, M), bf),
            pltpu.VMEM((M, H * D), bf),
            pltpu.VMEM((H * D, M), bf),
            pltpu.VMEM((_NB, Sk, Dc), bf),
            pltpu.VMEM((_NB, Hkv, W, D), bf),
            pltpu.VMEM((_NB, Hkv, W, D), bf),
            pltpu.VMEM((H * B, D), f32),
            pltpu.VMEM((Dc // 128, H * B, 128), f32),
            pltpu.VMEM((H * B, D), f32),
            pltpu.VMEM((Dc // 128, B * H, 128), f32),
            pltpu.VMEM((B * H, D), f32),
            pltpu.VMEM((H * B, D), f32),
            pltpu.SemaphoreType.DMA((2, _NCH)),
            pltpu.SemaphoreType.DMA((len(_TAIL) - 1,)),
        ],
        compiler_params=pltpu.CompilerParams(vmem_limit_bytes=80 * 2**20),
    )(
        A_x.reshape(B, M), A_c_kv,
        A_w_q.reshape(M * H, D), A_w_uk.reshape(Dc * H, D), A_w_uv.reshape(Dc * H, D),
        A_w_o.reshape(H * D, M), B_k_cache, B_v_cache, B_wq, B_wo, gate_w,
    )
    return out.reshape(B, Sq, M)
```

```python
import functools
import math

import jax
import jax.numpy as jnp
from jax import lax
import jax.experimental.pallas as pl
import jax.experimental.pallas.tpu as pltpu

_LOG2E = 1.4426950408889634
_NCH = 4
_NPC = 32
_NB = 2
_TAIL = (4, 2, 2)

_NT = (((1,), (1,)), ((), ()))


def _dot(a, b):
    return jnp.dot(a, b, preferred_element_type=jnp.float32)


def _dot_nt(a, b):
    return lax.dot_general(a, b, _NT, preferred_element_type=jnp.float32)


def _kernel(
    x_hbm, c_hbm, wq_hbm, wuk_hbm, wuv_hbm, wo_hbm, k_hbm, v_hbm, bwq_hbm, bwo_hbm, gw_hbm,
    o_ref,
    x_v, gw_v, wq_v, wuk_v, wuv_v, wo_v, bwq_v, bwo_v, c_v, k_v, v_v,
    qa_s, ql_s, qb_s, cl_s, ob_s, ctx_s,
    sems, tail_sems,
    *, B, H, D, M, Sk, Dc, Hkv, W,
):
    f32, bf16 = jnp.float32, jnp.bfloat16
    REP = H // Hkv
    CCH = Sk // _NCH
    CT = Dc // 128
    HP = H // 2
    HC = H // _NCH
    QC = HC * D

    class Chunk:
        def __init__(self, copy, pieces):
            self.copy = copy
            self.pieces = (pieces[:len(pieces) // 2], pieces[len(pieces) // 2:])

        def start(self, part=0, nparts=1):
            for queue, pieces in enumerate(self.pieces):
                n = len(pieces)
                for piece in pieces[part * n // nparts:(part + 1) * n // nparts]:
                    self.copy(*piece).start(priority=queue)

        def wait(self, issue=lambda part, nparts: None):
            for piece in self.pieces[0]:
                self.copy(*piece).wait()
            for part, piece in enumerate(self.pieces[1]):
                self.copy(*piece).wait()
                issue(part, len(self.pieces[1]))

    def row_pieces(n):
        return [(i * (n // _NPC), n // _NPC) for i in range(_NPC)]

    def rows_chunk(hbm, vmem, item, k):
        n = hbm.shape[0] // _NCH

        def copy(r0, rows):
            rng = pl.ds(pl.multiple_of(k * n + r0, math.gcd(n, r0)), rows)
            return pltpu.make_async_copy(hbm.at[rng], vmem.at[rng], sems.at[item % 2, k])
        return Chunk(copy, row_pieces(n))

    def wq_chunk(k): return rows_chunk(wq_hbm, wq_v, 0, k)
    def wuk_chunk(k): return rows_chunk(wuk_hbm, wuk_v, 1, k)
    def c_chunk(b, k): return rows_chunk(c_hbm.at[b], c_v.at[b % _NB], 2 + b, k)
    def wuv_chunk(k): return rows_chunk(wuv_hbm, wuv_v, 2 + B, k)
    def wo_chunk(k): return rows_chunk(wo_hbm, wo_v, 3 + B, k)
    def bwo_chunk(k): return rows_chunk(bwo_hbm, bwo_v, 5 + 2 * B, k)

    def bwq_chunk(k):
        cols = pl.ds(pl.multiple_of(k * QC, QC), QC)

        def copy(r0, rows):
            rng = pl.ds(r0, rows)
            return pltpu.make_async_copy(
                bwq_hbm.at[rng, cols], bwq_v.at[rng, cols], sems.at[(4 + B) % 2, k])
        return Chunk(copy, row_pieces(M))

    def kv_chunk(b, j):
        rows = 4 * W // _NPC

        def copy(hbm, vmem, g, r0):
            return pltpu.make_async_copy(
                hbm.at[b, 2 * j + g, pl.ds(Sk - W + r0, rows)],
                vmem.at[b % _NB, 2 * j + g, pl.ds(r0, rows)], sems.at[(5 + B + b) % 2, j])
        return Chunk(copy, [(hbm, vmem, g, r0)
                            for hbm, vmem in ((k_hbm, k_v), (v_hbm, v_v))
                            for g in range(2) for r0 in range(0, W, rows)])

    tail_h0 = [H - HC + sum(_TAIL[:i]) for i in range(len(_TAIL))]

    def bwo_tail(i):
        n = _TAIL[i] * D // 2

        def copy(r0):
            sem = sems.at[(5 + 2 * B) % 2, _NCH - 1] if i == 0 else tail_sems.at[i - 1]
            rng = pl.ds(tail_h0[i] * D + r0, n)
            return pltpu.make_async_copy(bwo_hbm.at[rng], bwo_v.at[rng], sem)
        return Chunk(copy, [(0,), (n,)])

    def start_tail(part, nparts):
        for i in range(len(_TAIL)):
            if part == i * nparts // len(_TAIL):
                bwo_tail(i).start()

    def in_order(n, start_fn):
        def body(i, carry):
            start_fn(i)
            return carry
        lax.fori_loop(0, n, body, 0)

    x_copy = pltpu.make_async_copy(x_hbm, x_v, tail_sems.at[0])
    gw_copy = pltpu.make_async_copy(gw_hbm, gw_v, tail_sems.at[1])
    x_copy.start()
    gw_copy.start()
    in_order(_NCH, lambda k: wq_chunk(k).start())

    def head_pairs(w_v, k):
        n = w_v.shape[0] // _NCH
        w = w_v[pl.ds(pl.multiple_of(k * n, n), n), :]
        u = pltpu.bitcast(w, jnp.uint32).reshape(n // H, HP, D)
        u = jnp.swapaxes(u, 0, 1)
        for p in range(HP):
            even = pltpu.bitcast(u[p] << 16, f32).astype(bf16)
            odd = pltpu.bitcast(u[p] & jnp.uint32(0xFFFF0000), f32).astype(bf16)
            yield 2 * p, even
            yield 2 * p + 1, odd

    def head_rows(h):
        return pl.ds(h * B, B)

    x_copy.wait()
    gw_copy.wait()

    qa_s[...] = jnp.zeros_like(qa_s)

    def qa_body(k, carry):
        wq_chunk(k).wait(wuk_chunk(k).start)
        xk = x_v[:, pl.ds(pl.multiple_of(k * 128, 128), 128)]
        for h, w in head_pairs(wq_v, k):
            qa_s[head_rows(h), :] += _dot(xk, w)
        return carry
    lax.fori_loop(0, _NCH, qa_body, 0)

    scale = (D ** -0.5) * _LOG2E

    def ql_body(k, carry):
        wuk_chunk(k).wait(c_chunk(0, k).start)
        for h, w in head_pairs(wuk_v, k):
            q = qa_s[head_rows(h), :].astype(bf16)
            ql_s[k, head_rows(h), :] = _dot_nt(q, w) * scale
        return carry
    lax.fori_loop(0, _NCH, ql_body, 0)

    def a_body(b, carry):
        q = jnp.concatenate(
            [ql_s[t, pl.ds(b, H, stride=B), :] for t in range(CT)], axis=-1
        ).astype(bf16)

        def chunk_body(k, mla):
            m_prev, l_prev, acc = mla
            pl.when(b + 1 < B)(lambda: c_chunk(b, k).wait(c_chunk(b + 1, k).start))
            pl.when(b + 1 == B)(lambda: c_chunk(b, k).wait(wuv_chunk(k).start))

            c = c_v[b % _NB, pl.ds(pl.multiple_of(k * CCH, CCH), CCH), :]
            s = _dot_nt(q, c)
            m_new = jnp.maximum(m_prev, jnp.max(s, axis=-1, keepdims=True))
            alpha = jnp.exp2(m_prev - m_new)
            p = jnp.exp2(s - m_new)
            l_new = alpha * l_prev + jnp.sum(p, axis=-1, keepdims=True)
            acc = alpha * acc + _dot(p.astype(bf16), c)
            return m_new, l_new, acc

        m0 = jnp.full((H, 1), -jnp.inf, f32)
        l0 = jnp.zeros((H, 1), f32)
        a0 = jnp.zeros((H, Dc), f32)
        _, l, acc = lax.fori_loop(0, _NCH, chunk_body, (m0, l0, a0))
        cl = acc / l
        for t in range(CT):
            cl_s[t, pl.ds(pl.multiple_of(b * H, H), H), :] = cl[:, t * 128:(t + 1) * 128]
        return carry

    lax.fori_loop(0, B, a_body, 0)

    ctx_s[...] = jnp.zeros_like(ctx_s)

    def ctx_body(k, carry):
        wuv_chunk(k).wait(wo_chunk(k).start)
        for h, w in head_pairs(wuv_v, k):
            lhs = cl_s[k, pl.ds(h, B, stride=H), :].astype(bf16)
            ctx_s[head_rows(h), :] += _dot(lhs, w)
        return carry
    lax.fori_loop(0, _NCH, ctx_body, 0)

    def out_proj(lhs_heads, w_v, k, acc):
        lhs = jnp.concatenate(lhs_heads, axis=-1).astype(bf16)
        n = w_v.shape[0] // _NCH
        return acc + _dot(lhs, w_v[pl.ds(pl.multiple_of(k * n, n), n), :])

    def oa_body(k, acc):
        wo_chunk(k).wait(bwq_chunk(k).start)
        lhs = [ctx_s[pl.ds(pl.multiple_of((k * HC + i) * B, B), B), :] for i in range(HC)]
        return out_proj(lhs, wo_v, k, acc)
    out_a = lax.fori_loop(0, _NCH, oa_body, jnp.zeros((B, M), f32))

    gate_logit = jnp.sum(x_v[...].astype(f32) * gw_v[...].astype(f32).reshape(1, M),
                         axis=-1, keepdims=True)
    gate = jax.nn.sigmoid(gate_logit)
    out_a = gate * out_a

    def qb_body(k, carry):
        bwq_chunk(k).wait(kv_chunk(0, k).start)
        q = _dot(x_v[...], bwq_v[:, pl.ds(pl.multiple_of(k * QC, QC), QC)]) * scale
        for i in range(HC):
            qb_s[pl.ds(pl.multiple_of((k * HC + i) * B, B), B), :] = q[:, i * D:(i + 1) * D]
        return carry
    lax.fori_loop(0, _NCH, qb_body, 0)

    first = lax.broadcasted_iota(jnp.int32, (2 * REP, 1), 0) < REP

    def b_body(b, carry):
        def pair_body(j, carry2):
            q8 = qb_s[pl.ds(j * 2 * REP * B + b, 2 * REP, stride=B), :].astype(bf16)
            pl.when(b + 1 < B)(lambda: kv_chunk(b, j).wait(kv_chunk(b + 1, j).start))
            pl.when((b + 1 == B) & (j + 1 < _NCH))(
                lambda: kv_chunk(b, j).wait(bwo_chunk(j).start))
            pl.when((b + 1 == B) & (j + 1 == _NCH))(lambda: kv_chunk(b, j).wait(start_tail))

            kk, vv = k_v.at[b % _NB], v_v.at[b % _NB]
            s = jnp.where(first, _dot_nt(q8, kk[2 * j]), _dot_nt(q8, kk[2 * j + 1]))
            m = jnp.max(s, axis=-1, keepdims=True)
            p = jnp.exp2(s - m)
            lb = jnp.sum(p, axis=-1, keepdims=True)
            pb = p.astype(bf16)
            o = jnp.where(first, _dot(pb, vv[2 * j]), _dot(pb, vv[2 * j + 1]))
            ob_s[pl.ds(pl.multiple_of(b * H + j * 2 * REP, 2 * REP), 2 * REP), :] = o / lb
            return carry2
        lax.fori_loop(0, _NCH, pair_body, 0)
        return carry

    lax.fori_loop(0, B, b_body, 0)

    def ob_heads(h0, n):
        return [ob_s[pl.ds(h0 + i, B, stride=H), :] for i in range(n)]

    def ob_body(k, acc):
        bwo_chunk(k).wait()
        return out_proj(ob_heads(k * HC, HC), bwo_v, k, acc)
    out_b = lax.fori_loop(0, _NCH - 1, ob_body, jnp.zeros((B, M), f32))
    for i, n in enumerate(_TAIL):
        lhs = jnp.concatenate(ob_heads(tail_h0[i], n), axis=-1).astype(bf16)
        bwo_tail(i).wait()
        out_b = out_b + _dot(lhs, bwo_v[pl.ds(tail_h0[i] * D, n * D), :])

    o_ref[...] = (out_a + (1.0 - gate) * out_b).astype(o_ref.dtype)


@jax.jit
def pallas_gated_mix__compressed_kv_cla__sliding_block_cached__decode_kernel(
    A_x: jax.Array,
    A_c_kv: jax.Array,
    A_w_q: jax.Array,
    A_w_uk: jax.Array,
    A_w_uv: jax.Array,
    A_w_o: jax.Array,
    B_x: jax.Array,
    B_k_cache: jax.Array,
    B_v_cache: jax.Array,
    B_wq: jax.Array,
    B_wo: jax.Array,
    gate_w: jax.Array,
):
    del B_x
    B, Sq, M = A_x.shape
    Sk, Dc = A_c_kv.shape[1], A_c_kv.shape[2]
    H, D = A_w_q.shape[1], A_w_q.shape[2]
    Hkv, Skb = B_k_cache.shape[1], B_k_cache.shape[2]
    W = min(4096, max(256, Skb // 4))
    assert Sq == 1 and B == 8 and D == 128 and Skb == Sk
    assert M == _NCH * 128 and Dc == _NCH * 128 and Hkv == 2 * _NCH and H == 4 * Hkv
    assert sum(_TAIL) == H // _NCH and len(_TAIL) >= 3 and _NB >= 2
    bf, f32 = jnp.bfloat16, jnp.float32

    kern = functools.partial(_kernel, B=B, H=H, D=D, M=M, Sk=Sk, Dc=Dc, Hkv=Hkv, W=W)
    out = pl.pallas_call(
        kern,
        out_shape=jax.ShapeDtypeStruct((B, M), A_x.dtype),
        in_specs=[pl.BlockSpec(memory_space=pl.ANY)] * 11,
        out_specs=pl.BlockSpec(memory_space=pltpu.VMEM),
        scratch_shapes=[
            pltpu.VMEM((B, M), bf),
            pltpu.VMEM((M,), bf),
            pltpu.VMEM((M * H, D), bf),
            pltpu.VMEM((Dc * H, D), bf),
            pltpu.VMEM((Dc * H, D), bf),
            pltpu.VMEM((H * D, M), bf),
            pltpu.VMEM((M, H * D), bf),
            pltpu.VMEM((H * D, M), bf),
            pltpu.VMEM((_NB, Sk, Dc), bf),
            pltpu.VMEM((_NB, Hkv, W, D), bf),
            pltpu.VMEM((_NB, Hkv, W, D), bf),
            pltpu.VMEM((H * B, D), f32),
            pltpu.VMEM((Dc // 128, H * B, 128), f32),
            pltpu.VMEM((H * B, D), f32),
            pltpu.VMEM((Dc // 128, B * H, 128), f32),
            pltpu.VMEM((B * H, D), f32),
            pltpu.VMEM((H * B, D), f32),
            pltpu.SemaphoreType.DMA((2, _NCH)),
            pltpu.SemaphoreType.DMA((len(_TAIL) - 1,)),
        ],
        compiler_params=pltpu.CompilerParams(vmem_limit_bytes=80 * 2**20),
    )(
        A_x.reshape(B, M), A_c_kv,
        A_w_q.reshape(M * H, D), A_w_uk.reshape(Dc * H, D), A_w_uv.reshape(Dc * H, D),
        A_w_o.reshape(H * D, M), B_k_cache, B_v_cache, B_wq, B_wo, gate_w,
    )
    return out.reshape(B, Sq, M)
```
